```python
import jax
import jax.numpy as jnp

def _softmax(x, axis=-1):
    return jax.nn.softmax(x, axis=axis)

def _gelu(x):
    return jax.nn.gelu(x, approximate=True)

def _silu(x):
    return jax.nn.silu(x)

def _sigmoid(x):
    return jax.nn.sigmoid(x)

def _layernorm(x, axis=-1, eps=1e-05):
    m = jnp.mean(x, axis=axis, keepdims=True)
    v = jnp.var(x, axis=axis, keepdims=True)
    return (x - m) / jnp.sqrt(v + eps)

def _scatter_add(tgt, idx, src, axis=0):
    return tgt.at[idx].add(src)

def _segment_sum(src, seg, n):
    return jax.ops.segment_sum(src, seg, n)

class _Rng:

    def __init__(self, key):
        self._k = key

    def _next(self):
        self._k, sub = jax.random.split(self._k)
        return sub

    def normal(self, shape):
        return jax.random.normal(self._next(), shape, dtype=jnp.bfloat16)

    def randint(self, lo, hi, shape):
        return jax.random.randint(self._next(), shape, lo, hi, dtype=jnp.int32)

    def uniform(self, shape, lo=0.0, hi=1.0):
        return jax.random.uniform(self._next(), shape, jnp.bfloat16, lo, hi)

    def permutation(self, n):
        return jax.random.permutation(self._next(), n)
kernel_name = 'adaLN_cond__grouped_kv_mqa__dense_activation_silu__prompt'

def _fwd_setup_inputs():
    _rng = _Rng(jax.random.key(int.from_bytes(__import__("os").urandom(4), "little")))
    _w = lambda a: (lambda t: t.astype(jnp.bfloat16) if jnp.issubdtype(t.dtype, jnp.floating) else t)(jnp.asarray(a))

    def _A_setup():
        B, S, D, H = (1, 2048, 640, 32)
        Dh = D // H
        return {'x': _w((lambda *s: _rng.normal(s) * 0.05)(B, S, D)), 'wq': _w((lambda *s: _rng.normal(s) * 0.05)(D, H * Dh)), 'wk': _w((lambda *s: _rng.normal(s) * 0.05)(D, Dh)), 'wv': _w((lambda *s: _rng.normal(s) * 0.05)(D, Dh)), 'wo': _w((lambda *s: _rng.normal(s) * 0.05)(H * Dh, D))}
    _A_in = _A_setup()

    def _B_setup():
        B, S, D, F = (1, 2048, 640, 1728)
        return {'x': _w((lambda *s: _rng.normal(s) * 0.05)(B, S, D)), 'w1': _w((lambda *s: _rng.normal(s) * 0.05)(D, F) * D ** (-0.5)), 'w2': _w((lambda *s: _rng.normal(s) * 0.05)(F, D) * F ** (-0.5))}
    _B_in = _B_setup()
    return {'A_x': _A_in['x'], 'A_wq': _A_in['wq'], 'A_wk': _A_in['wk'], 'A_wv': _A_in['wv'], 'A_wo': _A_in['wo'], 'B_x': _B_in['x'], 'B_w1': _B_in['w1'], 'B_w2': _B_in['w2'], 'c': _w((lambda *s: _rng.normal(s) * 0.05)(1, 640)), 'w_mod': _w((lambda *s: _rng.normal(s) * 0.05)(640, 6 * 640) * 640 ** (-0.5))}

def _fwd_reference(A_x, A_wq, A_wk, A_wv, A_wo, B_x, B_w1, B_w2, c, w_mod):

    def _A_ref(x, wq, wk, wv, wo):
        B, S, D = x.shape
        H = 32
        Dh = D // H
        q = (lambda x, *d: x.transpose(*d))((x @ wq).reshape(B, S, H, Dh), 0, 2, 1, 3)
        k = x @ wk
        v = x @ wv
        scores = jnp.einsum('bhqd,bkd->bhqk', q, k) * Dh ** (-0.5)
        p = _softmax(scores, axis=-1)
        o = jnp.einsum('bhqk,bkd->bhqd', p, v)
        return (lambda x, *d: x.transpose(*d))(o, 0, 2, 1, 3).reshape(B, S, H * Dh) @ wo

    def _B_ref(x, w1, w2):
        h = jnp.einsum('bsd,df->bsf', x, w1)
        h = _silu(h)
        out = jnp.einsum('bsf,fd->bsd', h, w2)
        return out
    x = A_x
    mod = (_silu(c) @ w_mod).reshape(c.shape[0], 6, 1, -1)
    sa, ca, ga, sb, cb, gb = (mod[:, 0].copy(), mod[:, 1].copy(), mod[:, 2].copy(), mod[:, 3].copy(), mod[:, 4].copy(), mod[:, 5].copy())
    h = _layernorm(x, axis=-1) * (1 + ca) + sa
    x = x + ga * _A_ref(h, A_wq, A_wk, A_wv, A_wo)
    h = _layernorm(x, axis=-1) * (1 + cb) + sb
    x = x + gb * _B_ref(h, B_w1, B_w2)
    return x

def setup_inputs():
    _inp = _fwd_setup_inputs()
    _gk = jax.random.fold_in(jax.random.key(int.from_bytes(__import__("os").urandom(4), "little")), 2 ** 31 - 1)
    _shapes = [[1, 2048, 640]]
    _dtypes = ['bfloat16']
    _gks = jax.random.split(_gk, len(_shapes))
    _gs = [jax.random.normal(k, s, dtype=jnp.dtype(d)) * 0.05 for k, s, d in zip(_gks, _shapes, _dtypes)]
    _inp['grad_out'] = _gs[0]
    return _inp

def reference(A_x, A_wq, A_wk, A_wv, A_wo, B_w1, B_w2, c, w_mod, B_x, grad_out):
    _const = dict(B_x=B_x)

    def _f(*_d):
        return _fwd_reference(**{'A_x': _d[0], 'A_wq': _d[1], 'A_wk': _d[2], 'A_wv': _d[3], 'A_wo': _d[4], 'B_w1': _d[5], 'B_w2': _d[6], 'c': _d[7], 'w_mod': _d[8], **_const})
    _out, _vjp = jax.vjp(_f, A_x, A_wq, A_wk, A_wv, A_wo, B_w1, B_w2, c, w_mod)
    _grads = _vjp(grad_out)
    _out0 = jnp.asarray(_out)
    return (_out0, *[jnp.asarray(_g) for _g in _grads])
```

```python
import math

import jax
import jax.numpy as jnp
from jax import lax
import jax.experimental.pallas as pl
import jax.experimental.pallas.tpu as pltpu

S, D, H, DH, F = 2048, 640, 32, 20, 1728
TQ = 256
NB = S // TQ
CK = 128
NCK = S // CK
NG = H // 4
EPS = 1e-5
f32, bf16, u32 = jnp.float32, jnp.bfloat16, jnp.uint32
LEAD = 2
SKEW = 4
NT = (((1,), (1,)), ((), ()))
SM_SCALE = DH ** (-0.5)
QSCALE = SM_SCALE * math.log2(math.e)
ONE_ROWS = ((30, 31), (30, 31), (30, 31), (0, 1))


def _dot(a, b):
    return jnp.dot(a, b, preferred_element_type=f32)


def _dot_nt(a, b):
    return lax.dot_general(a, b, NT, preferred_element_type=f32)


def _ln(x):
    mu = jnp.mean(x, axis=-1, keepdims=True)
    xc = x - mu
    var = jnp.mean(xc * xc, axis=-1, keepdims=True)
    rstd = lax.rsqrt(var + EPS)
    return xc * rstd, rstd


def _ln_bwd(dxhat, xhat, rstd):
    m1 = jnp.mean(dxhat, axis=-1, keepdims=True)
    m2 = jnp.mean(dxhat * xhat, axis=-1, keepdims=True)
    return rstd * (dxhat - m1 - xhat * m2)


def _colsum8(v):
    r, c = v.shape
    return jnp.sum(v.reshape(r // 8, 8, c), axis=0)


def _kernel(x_ref, wq_ref, wk_ref, wv_ref, wo_ref, w1_ref, w2_ref, c_ref, wmod_ref, g_ref,
            out_ref, dx_ref, dwq_ref, dwk_ref, dwv_ref, dwo_ref, dw1_ref, dw2_ref, dc_ref, dwmod_ref,
            mod_ref, h1_ref, qt_ref, kv_ref, kvt_ref, e_ref, s_ref, m_ref, ot_ref, dot_ref,
            linv_ref, dqt_ref, dx1_ref, dkv_ref, dw1_acc, dw2t_acc, dwo_acc, dmod_acc,
            wqt_ref, dkvc_ref, ds_ref):
    c = c_ref[...].astype(f32)
    sig_c = jax.nn.sigmoid(c)
    sc = c * sig_c
    mod_ref[...] = _dot(jnp.broadcast_to(sc, (8, D)).astype(bf16), wmod_ref[...])

    def modrow(k):
        return mod_ref[0:1, k * D:(k + 1) * D]

    wqt_ref[...] = wq_ref[...].T

    d_i = lax.broadcasted_iota(jnp.int32, (DH, 128), 0)
    n_i = lax.broadcasted_iota(jnp.int32, (DH, 128), 1)
    sel = jnp.where((n_i % 32) - 4 * (n_i // 32) == d_i, 1.0, 0.0).astype(bf16)
    wall = jnp.concatenate([_dot(wk_ref[...], sel), _dot(wv_ref[...], sel)], axis=1).astype(bf16)
    wallt = wall.T

    col = lax.broadcasted_iota(jnp.int32, (TQ, 256), 1)
    row = lax.broadcasted_iota(jnp.int32, (256, TQ), 0)

    def ones_mask(idx):
        m = None
        for r in range(4):
            for o in ONE_ROWS[r]:
                t = idx == (128 + 32 * r + o)
                m = t if m is None else jnp.logical_or(m, t)
        return m

    colmask = ones_mask(col)
    rowmask = ones_mask(row)
    sa, ca = modrow(0), modrow(1)
    for i in range(NB):
        rows = slice(i * TQ, (i + 1) * TQ)
        xhat, _ = _ln(x_ref[rows, :].astype(f32))
        h1 = (xhat * (1.0 + ca) + sa).astype(bf16)
        h1_ref[rows, :] = h1
        qt_ref[i] = (_dot_nt(wqt_ref[...], h1) * QSCALE).astype(bf16)
        kvt = jnp.where(rowmask, 1.0, _dot_nt(wallt, h1))
        kvt_ref[:, rows] = kvt.astype(bf16)
        kv = jnp.where(colmask, 1.0, _dot(h1, wall)).astype(bf16)
        for v in range(8):
            kv_ref[v, rows, :] = kv[:, 32 * v:32 * v + 32]

    dkv_ref[...] = jnp.zeros_like(dkv_ref)
    dw1_acc[...] = jnp.zeros_like(dw1_acc)
    dw2t_acc[...] = jnp.zeros_like(dw2t_acc)
    dwo_acc[...] = jnp.zeros_like(dwo_acc)
    dmod_acc[...] = jnp.zeros_like(dmod_acc)

    wrow = lax.broadcasted_iota(jnp.int32, (32, TQ), 0)

    def head_mask(r):
        return jnp.logical_and(wrow >= 4 * r, wrow < 4 * r + DH)

    def scores_chunk(j, r, qwin, slot, mrun):
        ks = slice(j * CK, (j + 1) * CK)
        s = _dot(kv_ref[r, ks, :], qwin)
        s_ref[slot, ks, :] = s
        cm = jnp.max(s.reshape(CK // 8, 8, TQ), axis=0)
        return cm if mrun is None else jnp.maximum(mrun, cm)

    def finish_max(mrun):
        return jnp.broadcast_to(jnp.max(mrun, axis=0, keepdims=True), (8, TQ))

    mrun = None
    qwin0 = qt_ref[0, 0:32, :]
    for j in range(NCK):
        mrun = scores_chunk(j, 0, qwin0, 0, mrun)
    m_ref[0] = finish_max(mrun)
    mrun = None
    qwin1 = qt_ref[0, 16:48, :]
    for j in range(LEAD):
        mrun = scores_chunk(j, 1, qwin1, 1, mrun)
    m_ref[1] = mrun

    def assemble(wins):
        pieces = []
        for p in range(5):
            t = None
            if p <= 3:
                t = wins[p][0:16]
            if p >= 1:
                u = wins[p - 1][16:32]
                t = u if t is None else t + u
            pieces.append(t)
        return jnp.concatenate(pieces, axis=0)

    def block_body(i, carry):
        rows = pl.ds(pl.multiple_of(i * TQ, TQ), TQ)

        def fwd_group(g, carry):
            base = pl.multiple_of(g * 80, 16)
            last = g == NG - 1
            nb_i = jnp.where(last, jnp.minimum(i + 1, NB - 1), i)
            nbase = pl.multiple_of(jnp.where(last, 0, base + 80), 16)

            def q_window(rr):
                if rr < 4:
                    return qt_ref[i, pl.ds(base + 16 * rr, 32), :]
                return qt_ref[nb_i, pl.ds(nbase + 16 * (rr - 4), 32), :]

            m_head = {0: m_ref[0]}
            mrun = m_ref[1]
            wins = []
            oacc = None
            for t in range(4 * NCK):
                r, j = divmod(t, NCK)
                ra, ja = divmod(t + NCK + LEAD, NCK)
                mrun = scores_chunk(ja, ra % 4, q_window(ra), ra % 2, mrun)
                if ja == NCK - 1:
                    m_head[ra] = finish_max(mrun)
                    mrun = None
                h = g * 4 + r
                ks = slice(j * CK, (j + 1) * CK)
                ks2 = slice(j * CK // 2, (j + 1) * CK // 2)
                e = jnp.exp2(s_ref[r % 2, ks, :] - m_head[r][0:1, :]).astype(bf16)
                e_ref[h, ks2, :] = pltpu.bitcast(e, u32)
                po = _dot(kvt_ref[128 + 32 * r:128 + 32 * r + 32, ks], e)
                oacc = po if oacc is None else oacc + po
                if j == NCK - 1:
                    lr = ONE_ROWS[r][0]
                    linv = 1.0 / oacc[lr:lr + 1, :]
                    linv_ref[h] = jnp.broadcast_to(linv, (8, TQ))
                    wins.append(jnp.where(head_mask(r), oacc * linv, 0.0))
                    oacc = None
            m_ref[0] = m_head[4]
            m_ref[1] = mrun
            ot_ref[pl.ds(base, 80), :] = assemble(wins)
            return carry

        lax.fori_loop(0, NG, fwd_group, 0)

        ga, sb, cb, gb = modrow(2), modrow(3), modrow(4), modrow(5)
        ot = ot_ref[...]
        otb = ot.astype(bf16)
        a = _dot(otb.T, wo_ref[...])
        x1 = x_ref[rows, :].astype(f32) + ga * a
        xhat2, rstd2 = _ln(x1)
        h2 = (xhat2 * (1.0 + cb) + sb).astype(bf16)
        u = _dot(h2, w1_ref[...])
        sig = jax.nn.sigmoid(u)
        sl = (u * sig).astype(bf16)
        f = _dot(sl, w2_ref[...])
        out_ref[rows, :] = (x1 + gb * f).astype(out_ref.dtype)
        g = g_ref[rows, :].astype(f32)
        dmod_acc[:, 5 * D:6 * D] += _colsum8(g * f)
        df = (g * gb).astype(bf16)
        dsl = _dot_nt(df, w2_ref[...])
        du = (dsl * (sig * (1.0 + u * (1.0 - sig)))).astype(bf16)
        dw2t_acc[...] += _dot(df.T, sl)
        dh2 = _dot_nt(du, w1_ref[...])
        dw1_acc[...] += _dot(h2.T, du)
        dmod_acc[:, 3 * D:4 * D] += _colsum8(dh2)
        dmod_acc[:, 4 * D:5 * D] += _colsum8(dh2 * xhat2)
        dx1 = g + _ln_bwd(dh2 * (1.0 + cb), xhat2, rstd2)
        dx1_ref[rows, :] = dx1
        dmod_acc[:, 2 * D:3 * D] += _colsum8(dx1 * a)
        da = (dx1 * ga).astype(bf16)
        dwo_acc[...] += _dot(otb, da)
        dot_ref[...] = _dot_nt(wo_ref[...], da)

        def bwd_group(g, carry):
            base = pl.multiple_of(g * 80, 16)
            gws = []
            for r in range(4):
                wsl = pl.ds(base + 16 * r, 32)
                dow = jnp.where(head_mask(r), dot_ref[wsl, :], 0.0)
                linv = linv_ref[g * 4 + r][0:1, :]
                delta = jnp.sum(dow * ot_ref[wsl, :], axis=0, keepdims=True) * linv
                d_hi = delta.astype(bf16).astype(f32)
                d_lo = delta - d_hi
                r0, r1 = ONE_ROWS[r]
                gw = dow * linv
                gw = jnp.where(wrow == r0, -d_hi, gw)
                gw = jnp.where(wrow == r1, -d_lo, gw)
                gws.append(gw.astype(bf16))
            wins = []
            dq = None
            for t in range(4 * NCK + SKEW):
                if t < 4 * NCK:
                    r, j = divmod(t, NCK)
                    ks = slice(j * CK, (j + 1) * CK)
                    ks2 = slice(j * CK // 2, (j + 1) * CK // 2)
                    gt = _dot(kv_ref[4 + r, ks, :], gws[r])
                    e = pltpu.bitcast(e_ref[g * 4 + r, ks2, :], bf16)
                    ds_ref[r % 2, ks2, :] = pltpu.bitcast((e.astype(f32) * gt).astype(bf16), u32)
                if t >= SKEW:
                    r, j = divmod(t - SKEW, NCK)
                    ks = slice(j * CK, (j + 1) * CK)
                    ks2 = slice(j * CK // 2, (j + 1) * CK // 2)
                    qwin = qt_ref[i, pl.ds(base + 16 * r, 32), :]
                    ds = pltpu.bitcast(ds_ref[r % 2, ks2, :], bf16)
                    e = pltpu.bitcast(e_ref[g * 4 + r, ks2, :], bf16)
                    pq = _dot(kvt_ref[32 * r:32 * r + 32, ks], ds)
                    dq = pq if dq is None else dq + pq
                    dkv_ref[32 * r:32 * r + 32, ks] += _dot_nt(qwin, ds)
                    dkv_ref[128 + 32 * r:128 + 32 * r + 32, ks] += _dot_nt(gws[r], e)
                    if j == NCK - 1:
                        wins.append(jnp.where(head_mask(r), dq * SM_SCALE, 0.0))
                        dq = None
            dqt_ref[i, pl.ds(base, 80), :] = assemble(wins).astype(bf16)
            return carry

        lax.fori_loop(0, NG, bwd_group, 0)
        return carry

    lax.fori_loop(0, NB, block_body, 0)

    dkt = None
    dvt = None
    for r in range(4):
        a_ = dkv_ref[36 * r:36 * r + DH, :]
        b_ = dkv_ref[128 + 36 * r:128 + 36 * r + DH, :]
        dkt = a_ if dkt is None else dkt + a_
        dvt = b_ if dvt is None else dvt + b_
    dkvc_ref[...] = jnp.zeros_like(dkvc_ref)
    dkvc_ref[0:DH, :] = dkt * (SM_SCALE / QSCALE)
    dkvc_ref[32:32 + DH, :] = dvt
    dkvc = dkvc_ref[...].astype(bf16)
    wkvc = jnp.concatenate([wall[:, 0:32], wall[:, 128:160]], axis=1)

    dwkv = _dot(dkvc, h1_ref[...]).T
    dwk_ref[...] = dwkv[:, 0:DH].astype(dwk_ref.dtype)
    dwv_ref[...] = dwkv[:, 32:32 + DH].astype(dwv_ref.dtype)

    dwqt = None
    for i in range(NB):
        rows = slice(i * TQ, (i + 1) * TQ)
        dqt = dqt_ref[i]
        t = _dot(dqt, h1_ref[rows, :])
        dwqt = t if dwqt is None else dwqt + t
        dh1 = (_dot(wq_ref[...], dqt) + _dot(wkvc, dkvc[:, rows])).T
        xhat, rstd = _ln(x_ref[rows, :].astype(f32))
        dmod_acc[:, 0:D] += _colsum8(dh1)
        dmod_acc[:, D:2 * D] += _colsum8(dh1 * xhat)
        dx = dx1_ref[rows, :] + _ln_bwd(dh1 * (1.0 + ca), xhat, rstd)
        dx_ref[rows, :] = dx.astype(dx_ref.dtype)
    dwq_ref[...] = dwqt.T.astype(dwq_ref.dtype)
    dwo_ref[...] = dwo_acc[...].astype(dwo_ref.dtype)
    dw1_ref[...] = dw1_acc[...].astype(dw1_ref.dtype)
    dw2_ref[...] = dw2t_acc[...].T.astype(dw2_ref.dtype)

    dmod = jnp.sum(dmod_acc[...], axis=0, keepdims=True)
    d_hi = dmod.astype(bf16)
    d_lo = (dmod - d_hi.astype(f32)).astype(bf16)
    r8 = lax.broadcasted_iota(jnp.int32, (16, 6 * D), 0)
    dm2 = jnp.where(r8 == 0, d_hi.astype(f32), jnp.where(r8 == 1, d_lo.astype(f32), 0.0)).astype(bf16)
    dsc = _dot_nt(dm2, wmod_ref[...])
    dsc = dsc[0:1] + dsc[1:2]
    dc_ref[...] = (dsc * (sig_c * (1.0 + c * (1.0 - sig_c)))).astype(dc_ref.dtype)
    sc_col = jnp.broadcast_to(sc, (128, D)).T
    for n in range(6 * D // 128):
        dwmod_ref[:, n * 128:(n + 1) * 128] = (sc_col * dmod[:, n * 128:(n + 1) * 128]).astype(dwmod_ref.dtype)


@jax.jit
def pallas_adaLN_cond__grouped_kv_mqa__dense_activation_silu__prompt_kernel(
    A_x: jax.Array,
    A_wq: jax.Array,
    A_wk: jax.Array,
    A_wv: jax.Array,
    A_wo: jax.Array,
    B_x: jax.Array,
    B_w1: jax.Array,
    B_w2: jax.Array,
    c: jax.Array,
    w_mod: jax.Array,
    grad_out: jax.Array,
):
    del B_x
    x = A_x.reshape(S, D)
    g = grad_out.reshape(S, D)
    sds = jax.ShapeDtypeStruct
    out_shape = (
        sds((S, D), bf16), sds((S, D), bf16),
        sds((D, D), bf16), sds((D, DH), bf16), sds((D, DH), bf16), sds((D, D), bf16),
        sds((D, F), bf16), sds((F, D), bf16), sds((1, D), bf16), sds((D, 6 * D), bf16),
    )
    scratch = [
        pltpu.VMEM((8, 6 * D), f32),
        pltpu.VMEM((S, D), bf16),
        pltpu.VMEM((NB, D, TQ), bf16),
        pltpu.VMEM((8, S, 32), bf16),
        pltpu.VMEM((256, S), bf16),
        pltpu.VMEM((H, S // 2, TQ), u32),
        pltpu.VMEM((2, S, TQ), f32),
        pltpu.VMEM((2, 8, TQ), f32),
        pltpu.VMEM((D, TQ), f32),
        pltpu.VMEM((D, TQ), f32),
        pltpu.VMEM((H, 8, TQ), f32),
        pltpu.VMEM((NB, D, TQ), bf16),
        pltpu.VMEM((S, D), f32),
        pltpu.VMEM((256, S), f32),
        pltpu.VMEM((D, F), f32),
        pltpu.VMEM((D, F), f32),
        pltpu.VMEM((D, D), f32),
        pltpu.VMEM((8, 6 * D), f32),
        pltpu.VMEM((D, D), bf16),
        pltpu.VMEM((64, S), f32),
        pltpu.VMEM((2, S // 2, TQ), u32),
    ]
    outs = pl.pallas_call(
        _kernel,
        out_shape=out_shape,
        scratch_shapes=scratch,
        compiler_params=pltpu.CompilerParams(vmem_limit_bytes=120 * 1024 * 1024),
    )(x, A_wq, A_wk, A_wv, A_wo, B_w1, B_w2, c, w_mod, g)
    out, dx = outs[0].reshape(1, S, D), outs[1].reshape(1, S, D)
    return (out, dx) + tuple(outs[2:])
```

```python
import math

import jax
import jax.numpy as jnp
from jax import lax
import jax.experimental.pallas as pl
import jax.experimental.pallas.tpu as pltpu

S, D, H, DH, F = 2048, 640, 32, 20, 1728
TQ = 256
NB = S // TQ
CK = 128
NCK = S // CK
HF = 4
HB = 8
EPS = 1e-5
f32, bf16, u32 = jnp.float32, jnp.bfloat16, jnp.uint32
LEAD = 4
SKEW = 3
NT = (((1,), (1,)), ((), ()))
SM_SCALE = DH ** (-0.5)
QSCALE = SM_SCALE * math.log2(math.e)
ONE_ROWS = ((30, 31), (30, 31), (30, 31), (0, 1))

SEM_X = 0
SEM_WMA, SEM_WMB, SEM_WQ, SEM_WO, SEM_W1, SEM_W2, SEM_G = range(NB, NB + 7)
SEM_OUT = NB + 7
SEM_DX = 2 * NB + 7
SEM_DWQ, SEM_DWO, SEM_DW1, SEM_DW2, SEM_DMA_, SEM_DMB = range(3 * NB + 7, 3 * NB + 13)
NSEM = 3 * NB + 13


def woff(rr):
    return 80 * (rr // 4) + 16 * (rr % 4)


def _pk(v):
    return pltpu.bitcast(v, u32)


def _upk(v):
    return pltpu.bitcast(v, bf16)


def _dot(a, b):
    return jnp.dot(a, b, preferred_element_type=f32)


def _dot_nt(a, b):
    return lax.dot_general(a, b, NT, preferred_element_type=f32)


def _ln(x):
    mu = jnp.mean(x, axis=-1, keepdims=True)
    xc = x - mu
    var = jnp.mean(xc * xc, axis=-1, keepdims=True)
    rstd = lax.rsqrt(var + EPS)
    return xc * rstd, rstd


def _ln_bwd(dxhat, xhat, rstd):
    m1 = jnp.mean(dxhat, axis=-1, keepdims=True)
    m2 = jnp.mean(dxhat * xhat, axis=-1, keepdims=True)
    return rstd * (dxhat - m1 - xhat * m2)


def _colsum8(v):
    r, c = v.shape
    return jnp.sum(v.reshape(r // 8, 8, c), axis=0)


def _kernel(x_hbm, wq_hbm, wkt_ref, wvt_ref, wo_hbm, w1t_hbm, w2_hbm, c_ref, wmod_hbm, g_hbm,
            out_hbm, dx_hbm, dwq_hbm, dwkt_ref, dwvt_ref, dwo_hbm, dw1t_hbm, dw2_hbm, dc_ref, dwmod_hbm,
            x_ref, g_ref, wq_ref, wo_ref, w1t_ref, w2_ref, wmod_ref,
            out_v, dwq_v, dwo_v, dw1t_v, dw2_v, dwmod_v,
            mod_ref, h1_ref, qt_ref, kv_ref, kvt_ref, e_ref, s_ref, m_ref, ot_ref, gw_ref,
            linv_ref, dqt_ref, dx1_ref, dkv_ref, dw1t_acc, dw2_acc, dwo_acc, dmod_acc,
            wqt_ref, dkvc_ref, ds_ref, wkvc_ref, sccol_ref, xh_ref, xt_acc, qs_acc, sems):

    def blk(i):
        return pl.ds(pl.multiple_of(i * TQ, TQ), TQ)

    def x_copy(i):
        return pltpu.make_async_copy(x_hbm.at[blk(i)], x_ref.at[blk(i)], sems.at[SEM_X + i])

    def out_copy(i):
        return pltpu.make_async_copy(out_v.at[blk(i)], out_hbm.at[blk(i)], sems.at[SEM_OUT + i])

    def dx_copy(i):
        return pltpu.make_async_copy(g_ref.at[blk(i)], dx_hbm.at[blk(i)], sems.at[SEM_DX + i])

    cp_wma = pltpu.make_async_copy(wmod_hbm.at[:, 0:2 * D], wmod_ref.at[:, 0:2 * D], sems.at[SEM_WMA])
    cp_wmb = pltpu.make_async_copy(wmod_hbm.at[:, 2 * D:6 * D], wmod_ref.at[:, 2 * D:6 * D], sems.at[SEM_WMB])
    cp_wq = pltpu.make_async_copy(wq_hbm, wq_ref, sems.at[SEM_WQ])
    cp_wo = pltpu.make_async_copy(wo_hbm, wo_ref, sems.at[SEM_WO])
    cp_w1 = pltpu.make_async_copy(w1t_hbm, w1t_ref, sems.at[SEM_W1])
    cp_w2 = pltpu.make_async_copy(w2_hbm, w2_ref, sems.at[SEM_W2])
    cp_g = pltpu.make_async_copy(g_hbm, g_ref, sems.at[SEM_G])
    cp_dwq = pltpu.make_async_copy(dwq_v, dwq_hbm, sems.at[SEM_DWQ])
    cp_dwo = pltpu.make_async_copy(dwo_v, dwo_hbm, sems.at[SEM_DWO])
    cp_dw1 = pltpu.make_async_copy(dw1t_v, dw1t_hbm, sems.at[SEM_DW1])
    cp_dw2 = pltpu.make_async_copy(dw2_v, dw2_hbm, sems.at[SEM_DW2])
    cp_dma = pltpu.make_async_copy(dwmod_v.at[:, 0:2 * D], dwmod_hbm.at[:, 0:2 * D], sems.at[SEM_DMA_])
    cp_dmb = pltpu.make_async_copy(dwmod_v.at[:, 2 * D:6 * D], dwmod_hbm.at[:, 2 * D:6 * D], sems.at[SEM_DMB])

    cp_wma.start()
    cp_wq.start()
    for i in range(NB):
        x_copy(i).start()

    def zero_body(k, carry):
        fr = pl.ds(pl.multiple_of(k * (F // 8), 8), F // 8)
        dr = pl.ds(pl.multiple_of(k * (D // 8), 8), D // 8)
        dkv_ref[pl.ds(pl.multiple_of(k * 32, 8), 32), :] = jnp.zeros((32, S), f32)
        dw1t_acc[fr, :] = jnp.zeros((F // 8, D), f32)
        dw2_acc[fr, :] = jnp.zeros((F // 8, D), f32)
        dwo_acc[dr, :] = jnp.zeros((D // 8, D), f32)
        xt_acc[dr, :] = jnp.zeros((D // 8, D), f32)
        qs_acc[dr, :] = jnp.zeros((D // 8, TQ), f32)
        return carry

    lax.fori_loop(0, 8, zero_body, 0)
    dmod_acc[...] = jnp.zeros_like(dmod_acc)
    gw_ref[H] = jnp.zeros((16, TQ), u32)

    c = c_ref[...].astype(f32)
    sig_c = jax.nn.sigmoid(c)
    sc = c * sig_c
    sc8 = jnp.broadcast_to(sc, (8, D)).astype(bf16)
    sccol_ref[...] = jnp.broadcast_to(sc, (128, D)).T

    r_i = lax.broadcasted_iota(jnp.int32, (64, DH), 0)
    d_i = lax.broadcasted_iota(jnp.int32, (64, DH), 1)
    selk = jnp.where(r_i == d_i, 1.0, 0.0).astype(bf16)
    selv = jnp.where(r_i == d_i + 32, 1.0, 0.0).astype(bf16)
    wkvct = (_dot(selk, wkt_ref[...]) + _dot(selv, wvt_ref[...])).astype(bf16)
    wkvc_ref[...] = wkvct.T
    sr = lax.broadcasted_iota(jnp.int32, (64, 256), 0)
    scn = lax.broadcasted_iota(jnp.int32, (64, 256), 1)
    shift = jnp.where(jnp.logical_and((scn // 128) == (sr // 32),
                                      (scn % 32) - 4 * ((scn % 128) // 32) == (sr % 32)), 1.0, 0.0)
    shift_t = shift.T.astype(bf16)
    shift = shift.astype(bf16)

    def ones_mask(idx):
        m = None
        for r in range(4):
            for o in ONE_ROWS[r]:
                t = idx == (128 + 32 * r + o)
                m = t if m is None else jnp.logical_or(m, t)
        return m

    colmask = ones_mask(lax.broadcasted_iota(jnp.int32, (TQ, 256), 1))
    rowmask = ones_mask(lax.broadcasted_iota(jnp.int32, (256, TQ), 0))

    cp_wq.wait()
    wqt_ref[...] = wq_ref[...].T
    cp_wma.wait()
    mod_ref[:, 0:2 * D] = _dot(sc8, wmod_ref[:, 0:2 * D])

    def modrow(k):
        return mod_ref[0:1, k * D:(k + 1) * D]

    def p0_ln(i):
        rows = blk(i)
        xhat, _ = _ln(x_ref[rows, :].astype(f32))
        xh_ref[rows, :] = xhat.astype(bf16)
        h1_ref[i % 2] = (xhat * (1.0 + modrow(1)) + modrow(0)).astype(bf16)

    def p0_body(i, carry):
        @pl.when(i + 1 < NB)
        def _():
            x_copy(i + 1).wait()

        h1 = h1_ref[i % 2]
        qt_ref[i] = _pk((_dot_nt(wqt_ref[...], h1) * QSCALE).astype(bf16))
        kvct = _dot_nt(wkvct, h1).astype(bf16)
        kvt_ref[i] = _pk(jnp.where(rowmask, 1.0, _dot(shift_t, kvct)).astype(bf16))
        kv = _pk(jnp.where(colmask, 1.0, _dot(kvct.T, shift)).astype(bf16))
        rows2 = pl.ds(pl.multiple_of(i * (TQ // 2), TQ // 2), TQ // 2)
        for v in range(8):
            kv_ref[v, rows2, :] = kv[:, 32 * v:32 * v + 32]
        p0_ln(jnp.where(i + 1 < NB, i + 1, i - 1))
        return carry

    x_copy(0).wait()
    p0_ln(0)
    cp_wmb.start()
    cp_wo.start()
    cp_w1.start()
    cp_w2.start()
    cp_g.start()
    lax.fori_loop(0, NB, p0_body, 0)

    wrow = lax.broadcasted_iota(jnp.int32, (32, TQ), 0)

    def head_mask(r):
        return jnp.logical_and(wrow >= 4 * r, wrow < 4 * r + DH)

    def kvt_chunk(v, j):
        return _upk(kvt_ref[j // 2, 16 * v:16 * v + 16, (j % 2) * CK:(j % 2 + 1) * CK])

    def scores_chunk(j, r, qwin, slot, mrun):
        ks = slice(j * CK, (j + 1) * CK)
        s = _dot(_upk(kv_ref[r, j * CK // 2:(j + 1) * CK // 2, :]), qwin)
        s_ref[slot, ks, :] = s
        cm = jnp.max(s.reshape(CK // 8, 8, TQ), axis=0)
        return cm if mrun is None else jnp.maximum(mrun, cm)

    def finish_max(mrun):
        return jnp.broadcast_to(jnp.max(mrun, axis=0, keepdims=True), (8, TQ))

    mrun = None
    qwin0 = _upk(qt_ref[0, 0:16, :])
    for j in range(NCK):
        mrun = scores_chunk(j, 0, qwin0, 0, mrun)
    m_ref[0] = finish_max(mrun)
    mrun = None
    qwin1 = _upk(qt_ref[0, 8:24, :])
    for j in range(LEAD):
        mrun = scores_chunk(j, 1, qwin1, 1, mrun)
    m_ref[1] = mrun

    def assemble(wins):
        pieces = []
        for p in range(5):
            t = None
            if p <= 3:
                t = wins[p][0:16]
            if p >= 1:
                u = wins[p - 1][16:32]
                t = u if t is None else t + u
            pieces.append(t)
        return jnp.concatenate(pieces, axis=0)

    def ds_produce(h, hg, r, j):
        ks = slice(j * CK, (j + 1) * CK)
        ks2 = slice(j * CK // 2, (j + 1) * CK // 2)
        gw = _upk(gw_ref[hg])
        e = _upk(e_ref[h, ks2, :])
        dkv_ref[128 + 32 * r:128 + 32 * r + 32, ks] += _dot_nt(gw, e)
        gt = _dot(_upk(kv_ref[4 + r, ks2, :]), gw)
        ds_ref[r % 2, ks2, :] = _pk((e.astype(f32) * gt).astype(bf16))

    def block_body(i, carry):
        rows = blk(i)

        def fwd_group(g, carry):
            base = pl.multiple_of(g * (20 * HF), 16)
            base2 = pl.multiple_of(g * (10 * HF), 8)
            last = g == H // HF - 1
            nb_i = jnp.where(last, jnp.minimum(i + 1, NB - 1), i)
            nbase2 = pl.multiple_of(jnp.where(last, 0, base2 + 10 * HF), 8)

            def q_window(rr):
                if rr < HF:
                    return _upk(qt_ref[i, pl.ds(base2 + woff(rr) // 2, 16), :])
                return _upk(qt_ref[nb_i, pl.ds(nbase2 + woff(rr - HF) // 2, 16), :])

            m_head = {0: m_ref[0]}
            mrun = m_ref[1]
            wins = []
            oacc = None
            for t in range(HF * NCK):
                rr, j = divmod(t, NCK)
                r = rr % 4
                ra, ja = divmod(t + NCK + LEAD, NCK)
                mrun = scores_chunk(ja, ra % 4, q_window(ra), ra % 2, mrun)
                if ja == NCK - 1:
                    m_head[ra] = finish_max(mrun)
                    mrun = None
                h = g * HF + rr
                ks = slice(j * CK, (j + 1) * CK)
                ks2 = slice(j * CK // 2, (j + 1) * CK // 2)
                e = jnp.exp2(s_ref[r % 2, ks, :] - m_head[rr][0:1, :]).astype(bf16)
                e_ref[h, ks2, :] = _pk(e)
                po = _dot(kvt_chunk(4 + r, j), e)
                oacc = po if oacc is None else oacc + po
                if j == NCK - 1:
                    lr = ONE_ROWS[r][0]
                    linv = 1.0 / oacc[lr:lr + 1, :]
                    linv_ref[h] = jnp.broadcast_to(linv, (8, TQ))
                    wins.append(jnp.where(head_mask(r), oacc * linv, 0.0))
                    oacc = None
                    if r == 3:
                        ot_ref[pl.ds(base + 80 * (rr // 4), 80), :] = assemble(wins)
                        wins = []
            m_ref[0] = m_head[HF]
            m_ref[1] = mrun
            return carry

        lax.fori_loop(0, H // HF, fwd_group, 0)

        @pl.when(i == 0)
        def _():
            cp_wmb.wait()
            cp_wo.wait()
            cp_w1.wait()
            cp_w2.wait()
            cp_g.wait()
            mod_ref[:, 2 * D:6 * D] = _dot(sc8, wmod_ref[:, 2 * D:6 * D])

        ga, sb, cb, gb = modrow(2), modrow(3), modrow(4), modrow(5)
        ot = ot_ref[...]
        otb = ot.astype(bf16)
        a = _dot(otb.T, wo_ref[...])
        g = g_ref[rows, :].astype(f32)
        df = (g * gb).astype(bf16)
        dsl = _dot_nt(df, w2_ref[...])
        x1 = x_ref[rows, :].astype(f32) + ga * a
        xhat2, rstd2 = _ln(x1)
        h2 = (xhat2 * (1.0 + cb) + sb).astype(bf16)
        u = _dot_nt(h2, w1t_ref[...])
        sig = jax.nn.sigmoid(u)
        sl = (u * sig).astype(bf16)
        du = (dsl * (sig * (1.0 + u * (1.0 - sig)))).astype(bf16)
        dh2 = _dot(du, w1t_ref[...])
        f = _dot(sl, w2_ref[...])
        out_v[rows, :] = (x1 + gb * f).astype(bf16)
        out_copy(i).start()
        dmod_acc[:, 5 * D:6 * D] += _colsum8(g * f)
        dmod_acc[:, 3 * D:4 * D] += _colsum8(dh2)
        dmod_acc[:, 4 * D:5 * D] += _colsum8(dh2 * xhat2)
        dx1 = g + _ln_bwd(dh2 * (1.0 + cb), xhat2, rstd2)
        dx1_ref[rows, :] = dx1
        dmod_acc[:, 2 * D:3 * D] += _colsum8(dx1 * a)
        da = (dx1 * ga).astype(bf16)
        dot = _dot_nt(wo_ref[...], da)
        dw2_acc[...] += _dot(sl.T, df)
        dw1t_acc[...] += _dot(du.T, h2)
        dwo_acc[...] += _dot(otb, da)
        for h in range(H):
            gg, r = divmod(h, 4)
            wsl = slice(80 * gg + 16 * r, 80 * gg + 16 * r + 32)
            dow = jnp.where(head_mask(r), dot[wsl, :], 0.0)
            linv = linv_ref[h][0:1, :]
            delta = jnp.sum(dow * ot[wsl, :], axis=0, keepdims=True) * linv
            d_hi = delta.astype(bf16).astype(f32)
            d_lo = delta - d_hi
            r0, r1 = ONE_ROWS[r]
            gw = dow * linv
            gw = jnp.where(wrow == r0, -d_hi, gw)
            gw = jnp.where(wrow == r1, -d_lo, gw)
            gw_ref[h] = _pk(gw.astype(bf16))
        for j in range(SKEW):
            ds_produce(0, 0, 0, j)

        @pl.when(i == NB - 1)
        def _():
            dmod_acc[0:1, 2 * D:6 * D] = jnp.sum(dmod_acc[:, 2 * D:6 * D], axis=0, keepdims=True)

            def stage(k, carry):
                fr = pl.ds(pl.multiple_of(k * (F // 4), 16), F // 4)
                dr = pl.ds(pl.multiple_of(k * (D // 4), 16), D // 4)
                dw1t_v[fr, :] = dw1t_acc[fr, :].astype(bf16)
                dw2_v[fr, :] = dw2_acc[fr, :].astype(bf16)
                dwo_v[dr, :] = dwo_acc[dr, :].astype(bf16)
                scc = sccol_ref[dr, :]
                for n in range(2 * D // 128, 6 * D // 128):
                    cs = slice(n * 128, (n + 1) * 128)
                    dwmod_v[dr, cs] = (scc * dmod_acc[0:1, cs]).astype(bf16)
                return carry

            lax.fori_loop(0, 4, stage, 0)
            cp_dw1.start()
            cp_dw2.start()
            cp_dwo.start()
            cp_dmb.start()

        def bwd_group(g, carry):
            base = pl.multiple_of(g * (20 * HB), 16)
            base2 = pl.multiple_of(g * (10 * HB), 8)
            hnext = jnp.minimum(g * HB + HB, H - 4)
            wins = []
            dq = None
            for t in range(HB * NCK):
                rp, jp = divmod(t + SKEW, NCK)
                ds_produce(g * HB + rp if rp < HB else hnext, g * HB + rp, rp % 4, jp)
                rr, j = divmod(t, NCK)
                r = rr % 4
                ks = slice(j * CK, (j + 1) * CK)
                ks2 = slice(j * CK // 2, (j + 1) * CK // 2)
                qwin = _upk(qt_ref[i, pl.ds(base2 + woff(rr) // 2, 16), :])
                ds = _upk(ds_ref[r % 2, ks2, :])
                dkv_ref[32 * r:32 * r + 32, ks] += _dot_nt(qwin, ds)
                pq = _dot(kvt_chunk(r, j), ds)
                dq = pq if dq is None else dq + pq
                if j == NCK - 1:
                    wins.append(jnp.where(head_mask(r), dq * SM_SCALE, 0.0))
                    dq = None
                    if r == 3:
                        dqt_ref[i, pl.ds(base + 80 * (rr // 4), 80), :] = assemble(wins).astype(bf16)
                        wins = []
            return carry

        lax.fori_loop(0, H // HB, bwd_group, 0)
        return carry

    lax.fori_loop(0, NB, block_body, 0)

    dkt = None
    dvt = None
    for r in range(4):
        a_ = dkv_ref[36 * r:36 * r + DH, :]
        b_ = dkv_ref[128 + 36 * r:128 + 36 * r + DH, :]
        dkt = a_ if dkt is None else dkt + a_
        dvt = b_ if dvt is None else dvt + b_
    dkv_ref[0:64, :] = jnp.zeros((64, S), f32)
    dkv_ref[0:DH, :] = dkt * (SM_SCALE / QSCALE)
    dkv_ref[32:32 + DH, :] = dvt
    dkvc = dkv_ref[0:64, :].astype(bf16)
    for i in range(NB):
        dkvc_ref[i] = dkvc[:, i * TQ:(i + 1) * TQ]

    sa, ca = modrow(0), modrow(1)
    yt = _dot(dkvc, xh_ref[...])
    ckv = jnp.sum(dkvc.astype(f32), axis=1, keepdims=True)
    dwkvt = yt * (1.0 + ca) + ckv * sa
    dwkt_ref[...] = dwkvt[0:DH, :].astype(bf16)
    dwvt_ref[...] = dwkvt[32:32 + DH, :].astype(bf16)

    def x_body(i, carry):
        dqt = dqt_ref[i]
        xt_acc[...] += _dot(dqt, xh_ref[blk(i), :])
        qs_acc[...] += dqt.astype(f32)
        return carry

    lax.fori_loop(0, NB, x_body, 0)
    xt = xt_acc[...]
    qs = qs_acc[...]
    cq = jnp.sum(qs, axis=1, keepdims=True)
    dwq_v[...] = (xt * (1.0 + ca) + cq * sa).T.astype(bf16)
    cp_dwq.start()
    wqt = wqt_ref[...].astype(f32)
    wkvf = wkvct.astype(f32)
    dsa = jnp.sum(wqt * cq, axis=0, keepdims=True) + jnp.sum(wkvf * ckv, axis=0, keepdims=True)
    dca = jnp.sum(wqt * xt, axis=0, keepdims=True) + jnp.sum(wkvf * yt, axis=0, keepdims=True)
    dmod = jnp.concatenate(
        [dsa, dca, dmod_acc[0:1, 2 * D:6 * D]], axis=1)
    for n in range(2 * D // 128):
        dwmod_v[:, n * 128:(n + 1) * 128] = (sccol_ref[...] * dmod[:, n * 128:(n + 1) * 128]).astype(bf16)
    cp_dma.start()

    d_hi = dmod.astype(bf16)
    d_lo = (dmod - d_hi.astype(f32)).astype(bf16)
    r8 = lax.broadcasted_iota(jnp.int32, (16, 6 * D), 0)
    dm2 = jnp.where(r8 == 0, d_hi.astype(f32), jnp.where(r8 == 1, d_lo.astype(f32), 0.0)).astype(bf16)
    dsc = _dot_nt(dm2, wmod_ref[...])
    dsc = dsc[0:1] + dsc[1:2]
    dc_ref[...] = (dsc * (sig_c * (1.0 + c * (1.0 - sig_c)))).astype(bf16)

    def fin_body(i, carry):
        rows = blk(i)
        dh1 = (_dot(wq_ref[...], dqt_ref[i]) + _dot(wkvc_ref[...], dkvc_ref[i])).T
        xhat, rstd = _ln(x_ref[rows, :].astype(f32))
        dx = dx1_ref[rows, :] + _ln_bwd(dh1 * (1.0 + modrow(1)), xhat, rstd)
        g_ref[rows, :] = dx.astype(bf16)
        dx_copy(i).start()
        return carry

    lax.fori_loop(0, NB, fin_body, 0)

    for i in range(NB):
        out_copy(i).wait()
        dx_copy(i).wait()
    cp_dw1.wait()
    cp_dw2.wait()
    cp_dwo.wait()
    cp_dmb.wait()
    cp_dma.wait()
    cp_dwq.wait()


@jax.jit
def pallas_adaLN_cond__grouped_kv_mqa__dense_activation_silu__prompt_kernel(
    A_x: jax.Array,
    A_wq: jax.Array,
    A_wk: jax.Array,
    A_wv: jax.Array,
    A_wo: jax.Array,
    B_x: jax.Array,
    B_w1: jax.Array,
    B_w2: jax.Array,
    c: jax.Array,
    w_mod: jax.Array,
    grad_out: jax.Array,
):
    del B_x
    x = A_x.reshape(S, D)
    g = grad_out.reshape(S, D)
    sds = jax.ShapeDtypeStruct
    out_shape = (
        sds((S, D), bf16), sds((S, D), bf16),
        sds((D, D), bf16), sds((DH, D), bf16), sds((DH, D), bf16), sds((D, D), bf16),
        sds((F, D), bf16), sds((F, D), bf16), sds((1, D), bf16), sds((D, 6 * D), bf16),
    )
    hbm = pl.BlockSpec(memory_space=pl.ANY)
    vm = pl.BlockSpec(memory_space=pltpu.VMEM)
    scratch = [
        pltpu.VMEM((S, D), bf16),
        pltpu.VMEM((S, D), bf16),
        pltpu.VMEM((D, D), bf16),
        pltpu.VMEM((D, D), bf16),
        pltpu.VMEM((F, D), bf16),
        pltpu.VMEM((F, D), bf16),
        pltpu.VMEM((D, 6 * D), bf16),
        pltpu.VMEM((S, D), bf16),
        pltpu.VMEM((D, D), bf16),
        pltpu.VMEM((D, D), bf16),
        pltpu.VMEM((F, D), bf16),
        pltpu.VMEM((F, D), bf16),
        pltpu.VMEM((D, 6 * D), bf16),
        pltpu.VMEM((8, 6 * D), f32),
        pltpu.VMEM((2, TQ, D), bf16),
        pltpu.VMEM((NB, D // 2, TQ), u32),
        pltpu.VMEM((8, S // 2, 32), u32),
        pltpu.VMEM((NB, 128, TQ), u32),
        pltpu.VMEM((H, S // 2, TQ), u32),
        pltpu.VMEM((2, S, TQ), f32),
        pltpu.VMEM((2, 8, TQ), f32),
        pltpu.VMEM((D, TQ), f32),
        pltpu.VMEM((H + 1, 16, TQ), u32),
        pltpu.VMEM((H, 8, TQ), f32),
        pltpu.VMEM((NB, D, TQ), bf16),
        pltpu.VMEM((S, D), f32),
        pltpu.VMEM((256, S), f32),
        pltpu.VMEM((F, D), f32),
        pltpu.VMEM((F, D), f32),
        pltpu.VMEM((D, D), f32),
        pltpu.VMEM((8, 6 * D), f32),
        pltpu.VMEM((D, D), bf16),
        pltpu.VMEM((NB, 64, TQ), bf16),
        pltpu.VMEM((2, S // 2, TQ), u32),
        pltpu.VMEM((D, 64), bf16),
        pltpu.VMEM((D, 128), f32),
        pltpu.VMEM((S, D), bf16),
        pltpu.VMEM((D, D), f32),
        pltpu.VMEM((D, TQ), f32),
        pltpu.SemaphoreType.DMA((NSEM,)),
    ]
    outs = pl.pallas_call(
        _kernel,
        out_shape=out_shape,
        in_specs=[hbm, hbm, vm, vm, hbm, hbm, hbm, vm, hbm, hbm],
        out_specs=(hbm, hbm, hbm, vm, vm, hbm, hbm, hbm, vm, hbm),
        scratch_shapes=scratch,
        compiler_params=pltpu.CompilerParams(vmem_limit_bytes=124 * 1024 * 1024),
    )(x, A_wq, A_wk.T, A_wv.T, A_wo, B_w1.T, B_w2, c, w_mod, g)
    out, dx, dwq, dwkt, dwvt, dwo, dw1t, dw2, dc, dwmod = outs
    return (out.reshape(1, S, D), dx.reshape(1, S, D), dwq, dwkt.T, dwvt.T, dwo, dw1t.T, dw2, dc, dwmod)
```

```python
import math

import jax
import jax.numpy as jnp
from jax import lax
import jax.experimental.pallas as pl
import jax.experimental.pallas.tpu as pltpu

S, D, H, DH, F = 2048, 640, 32, 20, 1728
TQ = 256
NB = S // TQ
CK = 128
NCK = S // CK
HF = 4
HB = 8
FS = 512
QS = 160
EPS = 1e-5
f32, bf16, u32 = jnp.float32, jnp.bfloat16, jnp.uint32
LEAD = 4
SKEW = 3
NT = (((1,), (1,)), ((), ()))
SM_SCALE = DH ** (-0.5)
QSCALE = SM_SCALE * math.log2(math.e)
ONE_ROWS = ((30, 31), (30, 31), (30, 31), (0, 1))

SEM_X = 0
SEM_WMA, SEM_WMB, SEM_WQ, SEM_WO, SEM_W1, SEM_W2, SEM_G = range(NB, NB + 7)
SEM_OUT = NB + 7
SEM_DX = 2 * NB + 7
SEM_DWQ, SEM_DWO, SEM_DW1, SEM_DW2, SEM_DMA_, SEM_DMB = range(3 * NB + 7, 3 * NB + 13)
NSEM = 3 * NB + 13


def woff(rr):
    return 80 * (rr // 4) + 16 * (rr % 4)


def _pk(v):
    return pltpu.bitcast(v, u32)


def _upk(v):
    return pltpu.bitcast(v, bf16)


def _dot(a, b):
    return jnp.dot(a, b, preferred_element_type=f32)


def _dot_nt(a, b):
    return lax.dot_general(a, b, NT, preferred_element_type=f32)


def _ln(x):
    mu = jnp.mean(x, axis=-1, keepdims=True)
    xc = x - mu
    var = jnp.mean(xc * xc, axis=-1, keepdims=True)
    rstd = lax.rsqrt(var + EPS)
    return xc * rstd, rstd


def _ln_bwd(dxhat, xhat, rstd):
    m1 = jnp.mean(dxhat, axis=-1, keepdims=True)
    m2 = jnp.mean(dxhat * xhat, axis=-1, keepdims=True)
    return rstd * (dxhat - m1 - xhat * m2)


def _hilo_rows(v):
    hi = v.astype(bf16).astype(f32)
    r = lax.broadcasted_iota(jnp.int32, (16, v.shape[1]), 0)
    return jnp.where(r == 0, hi, jnp.where(r == 1, v - hi, 0.0)).astype(bf16)


def _colsum8(v):
    r, c = v.shape
    return jnp.sum(v.reshape(r // 8, 8, c), axis=0)


def _kernel(x_hbm, wq_hbm, wkt_ref, wvt_ref, wo_hbm, w1t_hbm, w2_hbm, c_ref, wmod_hbm, g_hbm,
            out_hbm, dx_hbm, dwq_hbm, dwkt_ref, dwvt_ref, dwo_hbm, dw1t_hbm, dw2_hbm, dc_ref, dwmod_hbm,
            x_ref, g_ref, wq_ref, wo_ref, w1t_ref, w2_ref, wmod_ref,
            out_v, dwq_v, dwo_v, dw1t_v, dw2_v, dwmod_v,
            mod_ref, qt_ref, kv_ref, kvt_ref, e_ref, s_ref, m_ref, ot_ref, gw_ref,
            linv_ref, dqt_ref, dx1_ref, dkv_ref, dw1t_acc, dw2_acc, dwo_acc, dmod_acc,
            wqt_ref, dkvc_ref, ds_ref, wkvc_ref, sccol_ref, xh_ref, xt_acc, qs_acc, dscb_ref, sems):

    def blk(i):
        return pl.ds(pl.multiple_of(i * TQ, TQ), TQ)

    def x_copy(i):
        return pltpu.make_async_copy(x_hbm.at[blk(i)], x_ref.at[blk(i)], sems.at[SEM_X + i])

    def out_copy(i):
        return pltpu.make_async_copy(out_v.at[blk(i)], out_hbm.at[blk(i)], sems.at[SEM_OUT + i])

    def dx_copy(i):
        return pltpu.make_async_copy(g_ref.at[blk(i)], dx_hbm.at[blk(i)], sems.at[SEM_DX + i])

    cp_wma = pltpu.make_async_copy(wmod_hbm.at[:, 0:2 * D], wmod_ref.at[:, 0:2 * D], sems.at[SEM_WMA])
    cp_wmb = pltpu.make_async_copy(wmod_hbm.at[:, 2 * D:6 * D], wmod_ref.at[:, 2 * D:6 * D], sems.at[SEM_WMB])
    cp_wq = pltpu.make_async_copy(wq_hbm, wq_ref, sems.at[SEM_WQ])
    cp_wo = pltpu.make_async_copy(wo_hbm, wo_ref, sems.at[SEM_WO])
    cp_w1 = pltpu.make_async_copy(w1t_hbm, w1t_ref, sems.at[SEM_W1])
    cp_w2 = pltpu.make_async_copy(w2_hbm, w2_ref, sems.at[SEM_W2])
    cp_g = pltpu.make_async_copy(g_hbm, g_ref, sems.at[SEM_G])
    cp_dwq = pltpu.make_async_copy(dwq_v, dwq_hbm, sems.at[SEM_DWQ])
    cp_dwo = pltpu.make_async_copy(dwo_v, dwo_hbm, sems.at[SEM_DWO])
    cp_dw1 = pltpu.make_async_copy(dw1t_v, dw1t_hbm, sems.at[SEM_DW1])
    cp_dw2 = pltpu.make_async_copy(dw2_v, dw2_hbm, sems.at[SEM_DW2])
    cp_dma = pltpu.make_async_copy(dwmod_v.at[:, 0:2 * D], dwmod_hbm.at[:, 0:2 * D], sems.at[SEM_DMA_])
    cp_dmb = pltpu.make_async_copy(dwmod_v.at[:, 2 * D:6 * D], dwmod_hbm.at[:, 2 * D:6 * D], sems.at[SEM_DMB])

    cp_wq.start()
    cp_wma.start()
    x_copy(0).start()

    def zero_body(k, carry):
        fr = pl.ds(pl.multiple_of(k * (F // 8), 8), F // 8)
        dr = pl.ds(pl.multiple_of(k * (D // 8), 8), D // 8)
        dkv_ref[pl.ds(pl.multiple_of(k * 32, 8), 32), :] = jnp.zeros((32, S), f32)
        dw1t_acc[fr, :] = jnp.zeros((F // 8, D), f32)
        dw2_acc[fr, :] = jnp.zeros((F // 8, D), f32)
        dwo_acc[dr, :] = jnp.zeros((D // 8, D), f32)
        xt_acc[dr, :] = jnp.zeros((D // 8, D), f32)
        qs_acc[dr, :] = jnp.zeros((D // 8, TQ), f32)
        return carry

    lax.fori_loop(0, 8, zero_body, 0)
    dmod_acc[...] = jnp.zeros_like(dmod_acc)
    gw_ref[H] = jnp.zeros((16, TQ), u32)

    c = c_ref[...].astype(f32)
    sig_c = jax.nn.sigmoid(c)
    sc = c * sig_c
    sc8 = jnp.broadcast_to(sc, (8, D)).astype(bf16)
    sccol_ref[...] = jnp.broadcast_to(sc, (128, D)).T

    r_i = lax.broadcasted_iota(jnp.int32, (64, DH), 0)
    d_i = lax.broadcasted_iota(jnp.int32, (64, DH), 1)
    selk = jnp.where(r_i == d_i, 1.0, 0.0).astype(bf16)
    selv = jnp.where(r_i == d_i + 32, 1.0, 0.0).astype(bf16)
    wkvct = (_dot(selk, wkt_ref[...]) + _dot(selv, wvt_ref[...])).astype(bf16)
    wkvc_ref[...] = wkvct.T
    sr = lax.broadcasted_iota(jnp.int32, (64, 256), 0)
    scn = lax.broadcasted_iota(jnp.int32, (64, 256), 1)
    shift = jnp.where(jnp.logical_and((scn // 128) == (sr // 32),
                                      (scn % 32) - 4 * ((scn % 128) // 32) == (sr % 32)), 1.0, 0.0)
    shift_t = shift.T.astype(bf16)
    shift = shift.astype(bf16)

    def ones_mask(idx):
        m = None
        for r in range(4):
            for o in ONE_ROWS[r]:
                t = idx == (128 + 32 * r + o)
                m = t if m is None else jnp.logical_or(m, t)
        return m

    colmask = ones_mask(lax.broadcasted_iota(jnp.int32, (TQ, 256), 1))
    rowmask = ones_mask(lax.broadcasted_iota(jnp.int32, (256, TQ), 0))

    cp_wq.wait()
    for i in range(1, NB):
        x_copy(i).start()
    wqt_ref[...] = wq_ref[...].T
    cp_wma.wait()
    mod_ref[:, 0:2 * D] = _dot(sc8, wmod_ref[:, 0:2 * D])

    def modrow(k):
        return mod_ref[0:1, k * D:(k + 1) * D]

    def p0_ln(i):
        rows = blk(i)
        xhat, _ = _ln(x_ref[rows, :].astype(f32))
        xh_ref[rows, :] = xhat.astype(bf16)
        return (xhat * (1.0 + modrow(1)) + modrow(0)).astype(bf16)

    def p0_body(i, h1):
        @pl.when(i + 1 < NB)
        def _():
            x_copy(i + 1).wait()

        h1_next = p0_ln(jnp.minimum(i + 1, NB - 1))
        kvct = _dot_nt(wkvct, h1).astype(bf16)
        qt_ref.at[i][0:QS // 2, :] = _pk((_dot_nt(wqt_ref[0:QS, :], h1) * QSCALE).astype(bf16))
        kvt_ref.at[i][...] = _pk(jnp.where(rowmask, 1.0, _dot(shift_t, kvct)).astype(bf16))
        kv = _pk(jnp.where(colmask, 1.0, _dot(kvct.T, shift)).astype(bf16))
        rows2 = pl.ds(pl.multiple_of(i * (TQ // 2), TQ // 2), TQ // 2)
        for v in range(8):
            kv_ref[v, rows2, :] = kv[:, 32 * v:32 * v + 32]
        qt_ref.at[i][QS // 2:D // 2, :] = _pk((_dot_nt(wqt_ref[QS:D, :], h1) * QSCALE).astype(bf16))
        return h1_next

    x_copy(0).wait()
    h1_first = p0_ln(0)
    cp_wmb.start()
    cp_wo.start()
    cp_w1.start()
    cp_w2.start()
    cp_g.start()
    lax.fori_loop(0, NB, p0_body, h1_first)

    wrow = lax.broadcasted_iota(jnp.int32, (32, TQ), 0)

    def head_mask(r):
        return jnp.logical_and(wrow >= 4 * r, wrow < 4 * r + DH)

    def kvt_chunk(v, j):
        return _upk(kvt_ref[j // 2, 16 * v:16 * v + 16, (j % 2) * CK:(j % 2 + 1) * CK])

    def scores_chunk(j, r, qwin, slot, mrun):
        ks = slice(j * CK, (j + 1) * CK)
        s = _dot(_upk(kv_ref[r, j * CK // 2:(j + 1) * CK // 2, :]), qwin)
        s_ref[slot, ks, :] = s
        cm = jnp.max(s.reshape(CK // 8, 8, TQ), axis=0)
        return cm if mrun is None else jnp.maximum(mrun, cm)

    def finish_max(mrun):
        return jnp.broadcast_to(jnp.max(mrun, axis=0, keepdims=True), (8, TQ))

    mrun = None
    qwin0 = _upk(qt_ref[0, 0:16, :])
    for j in range(NCK):
        mrun = scores_chunk(j, 0, qwin0, 0, mrun)
    m_ref[0] = finish_max(mrun)
    mrun = None
    qwin1 = _upk(qt_ref[0, 8:24, :])
    for j in range(LEAD):
        mrun = scores_chunk(j, 1, qwin1, 1, mrun)
    m_ref[1] = mrun

    def assemble(wins):
        pieces = []
        for p in range(5):
            t = None
            if p <= 3:
                t = wins[p][0:16]
            if p >= 1:
                u = wins[p - 1][16:32]
                t = u if t is None else t + u
            pieces.append(t)
        return jnp.concatenate(pieces, axis=0)

    def ds_produce(h, hg, r, j):
        ks = slice(j * CK, (j + 1) * CK)
        ks2 = slice(j * CK // 2, (j + 1) * CK // 2)
        gw = _upk(gw_ref[hg])
        e = _upk(e_ref[h, ks2, :])
        dkv_ref[128 + 32 * r:128 + 32 * r + 32, ks] += _dot_nt(gw, e)
        gt = _dot(_upk(kv_ref[4 + r, ks2, :]), gw)
        ds_ref[r % 2, ks2, :] = _pk((e.astype(f32) * gt).astype(bf16))

    def block_body(i, carry):
        rows = blk(i)

        def fwd_group(g, carry):
            base = pl.multiple_of(g * (20 * HF), 16)
            base2 = pl.multiple_of(g * (10 * HF), 8)
            last = g == H // HF - 1
            nb_i = jnp.where(last, jnp.minimum(i + 1, NB - 1), i)
            nbase2 = pl.multiple_of(jnp.where(last, 0, base2 + 10 * HF), 8)

            def q_window(rr):
                if rr < HF:
                    return _upk(qt_ref[i, pl.ds(base2 + woff(rr) // 2, 16), :])
                return _upk(qt_ref[nb_i, pl.ds(nbase2 + woff(rr - HF) // 2, 16), :])

            m_head = {0: m_ref[0]}
            mrun = m_ref[1]
            wins = []
            oacc = None
            for t in range(HF * NCK):
                rr, j = divmod(t, NCK)
                r = rr % 4
                ra, ja = divmod(t + NCK + LEAD, NCK)
                mrun = scores_chunk(ja, ra % 4, q_window(ra), ra % 2, mrun)
                if ja == NCK - 1:
                    m_head[ra] = finish_max(mrun)
                    mrun = None
                h = g * HF + rr
                ks = slice(j * CK, (j + 1) * CK)
                ks2 = slice(j * CK // 2, (j + 1) * CK // 2)
                e = jnp.exp2(s_ref[r % 2, ks, :] - m_head[rr][0:1, :]).astype(bf16)
                e_ref[h, ks2, :] = _pk(e)
                po = _dot(kvt_chunk(4 + r, j), e)
                oacc = po if oacc is None else oacc + po
                if j == NCK - 1:
                    lr = ONE_ROWS[r][0]
                    linv = 1.0 / oacc[lr:lr + 1, :]
                    linv_ref[h] = jnp.broadcast_to(linv, (8, TQ))
                    wins.append(jnp.where(head_mask(r), oacc * linv, 0.0))
                    oacc = None
                    if r == 3:
                        ot_ref[pl.ds(base + 80 * (rr // 4), 80), :] = assemble(wins)
                        wins = []
            m_ref[0] = m_head[HF]
            m_ref[1] = mrun
            return carry

        lax.fori_loop(0, H // HF, fwd_group, 0)

        @pl.when(i == 0)
        def _():
            cp_wmb.wait()
            cp_wo.wait()
            cp_w1.wait()
            cp_w2.wait()
            cp_g.wait()
            mod_ref[:, 2 * D:6 * D] = _dot(sc8, wmod_ref[:, 2 * D:6 * D])

        ga, sb, cb, gb = modrow(2), modrow(3), modrow(4), modrow(5)
        g = g_ref[rows, :].astype(f32)
        df = (g * gb).astype(bf16)
        dsl_a = _dot_nt(df, w2_ref[0:FS, :])
        ot = ot_ref[...]
        otb = ot.astype(bf16)
        a = _dot(otb.T, wo_ref[...])
        dsl = jnp.concatenate([dsl_a, _dot_nt(df, w2_ref[FS:F, :])], axis=1)
        x1 = x_ref[rows, :].astype(f32) + ga * a
        xhat2, rstd2 = _ln(x1)
        h2 = (xhat2 * (1.0 + cb) + sb).astype(bf16)
        u = _dot_nt(h2, w1t_ref[...])
        sig = 0.5 * jnp.tanh(0.5 * u) + 0.5
        sl = (u * sig).astype(bf16)
        du = (dsl * (sig * (1.0 + u * (1.0 - sig)))).astype(bf16)
        dh2 = _dot(du, w1t_ref[...])
        f = _dot(sl, w2_ref[...])
        out_v[rows, :] = (x1 + gb * f).astype(bf16)
        out_copy(i).start()
        dmod_acc[:, 5 * D:6 * D] += _colsum8(g * f)
        dmod_acc[:, 3 * D:4 * D] += _colsum8(dh2)
        dmod_acc[:, 4 * D:5 * D] += _colsum8(dh2 * xhat2)
        dx1 = g + _ln_bwd(dh2 * (1.0 + cb), xhat2, rstd2)
        dx1_ref[rows, :] = dx1
        dmod_acc[:, 2 * D:3 * D] += _colsum8(dx1 * a)
        da = (dx1 * ga).astype(bf16)
        dot = _dot_nt(wo_ref[...], da)
        dw2_acc[...] += _dot(sl.T, df)
        dw1t_acc[...] += _dot(du.T, h2)
        for h in range(H):
            gg, r = divmod(h, 4)
            wsl = slice(80 * gg + 16 * r, 80 * gg + 16 * r + 32)
            dow = jnp.where(head_mask(r), dot[wsl, :], 0.0)
            linv = linv_ref[h][0:1, :]
            delta = jnp.sum(dow * ot[wsl, :], axis=0, keepdims=True) * linv
            d_hi = delta.astype(bf16).astype(f32)
            d_lo = delta - d_hi
            r0, r1 = ONE_ROWS[r]
            gw = dow * linv
            gw = jnp.where(wrow == r0, -d_hi, gw)
            gw = jnp.where(wrow == r1, -d_lo, gw)
            gw_ref.at[h][...] = _pk(gw.astype(bf16))
        for j in range(SKEW):
            ds_produce(0, 0, 0, j)
        dwo_acc[...] += _dot(otb, da)

        @pl.when(i == NB - 1)
        def _():
            dmb = jnp.sum(dmod_acc[:, 2 * D:6 * D], axis=0, keepdims=True)
            dmod_acc[0:1, 2 * D:6 * D] = dmb
            dmb2 = _hilo_rows(dmb)

            def stage(k, carry):
                fr = pl.ds(pl.multiple_of(k * (F // 4), 16), F // 4)
                dr = pl.ds(pl.multiple_of(k * (D // 4), 16), D // 4)
                dw1t_v[fr, :] = dw1t_acc[fr, :].astype(bf16)
                dw2_v[fr, :] = dw2_acc[fr, :].astype(bf16)
                dwo_v[dr, :] = dwo_acc[dr, :].astype(bf16)
                dscb_ref[k] = _dot_nt(dmb2, wmod_ref[dr, 2 * D:6 * D])
                scc = sccol_ref[dr, :]
                for n in range(2 * D // 128, 6 * D // 128):
                    cs = slice(n * 128, (n + 1) * 128)
                    dwmod_v[dr, cs] = (scc * dmod_acc[0:1, cs]).astype(bf16)
                return carry

            lax.fori_loop(0, 4, stage, 0)
            cp_dw1.start()
            cp_dw2.start()
            cp_dwo.start()
            cp_dmb.start()

        def bwd_group(g, carry):
            base = pl.multiple_of(g * (20 * HB), 16)
            base2 = pl.multiple_of(g * (10 * HB), 8)
            hnext = jnp.minimum(g * HB + HB, H - 4)
            wins = []
            dq = None
            for t in range(HB * NCK):
                rp, jp = divmod(t + SKEW, NCK)
                ds_produce(g * HB + rp if rp < HB else hnext, g * HB + rp, rp % 4, jp)
                rr, j = divmod(t, NCK)
                r = rr % 4
                ks = slice(j * CK, (j + 1) * CK)
                ks2 = slice(j * CK // 2, (j + 1) * CK // 2)
                qwin = _upk(qt_ref[i, pl.ds(base2 + woff(rr) // 2, 16), :])
                ds = _upk(ds_ref[r % 2, ks2, :])
                dkv_ref[32 * r:32 * r + 32, ks] += _dot_nt(qwin, ds)
                pq = _dot(kvt_chunk(r, j), ds)
                dq = pq if dq is None else dq + pq
                if j == NCK - 1:
                    wins.append(jnp.where(head_mask(r), dq * SM_SCALE, 0.0))
                    dq = None
                    if r == 3:
                        dqt_ref[i, pl.ds(base + 80 * (rr // 4), 80), :] = assemble(wins).astype(bf16)
                        wins = []
            return carry

        lax.fori_loop(0, H // HB, bwd_group, 0)
        return carry

    lax.fori_loop(0, NB, block_body, 0)

    dkt = None
    dvt = None
    for r in range(4):
        a_ = dkv_ref[36 * r:36 * r + DH, :]
        b_ = dkv_ref[128 + 36 * r:128 + 36 * r + DH, :]
        dkt = a_ if dkt is None else dkt + a_
        dvt = b_ if dvt is None else dvt + b_
    dkv_ref[0:64, :] = jnp.zeros((64, S), f32)
    dkv_ref[0:DH, :] = dkt * (SM_SCALE / QSCALE)
    dkv_ref[32:32 + DH, :] = dvt
    dkvc = dkv_ref[0:64, :].astype(bf16)
    for i in range(NB):
        dkvc_ref[i] = dkvc[:, i * TQ:(i + 1) * TQ]

    sa, ca = modrow(0), modrow(1)
    yt = _dot(dkvc, xh_ref[...])
    ckv = jnp.sum(dkvc.astype(f32), axis=1, keepdims=True)
    dwkvt = yt * (1.0 + ca) + ckv * sa
    dwkt_ref[...] = dwkvt[0:DH, :].astype(bf16)
    dwvt_ref[...] = dwkvt[32:32 + DH, :].astype(bf16)

    def x_body(i, carry):
        dqt = dqt_ref[i]
        xt_acc[...] += _dot(dqt, xh_ref[blk(i), :])
        qs_acc[...] += dqt.astype(f32)
        return carry

    lax.fori_loop(0, NB, x_body, 0)
    xt = xt_acc[...]
    qs = qs_acc[...]
    cq = jnp.sum(qs, axis=1, keepdims=True)
    dwq_v[...] = (xt * (1.0 + ca) + cq * sa).T.astype(bf16)
    cp_dwq.start()
    wqt = wqt_ref[...].astype(f32)
    wkvf = wkvct.astype(f32)
    dsa = jnp.sum(wqt * cq, axis=0, keepdims=True) + jnp.sum(wkvf * ckv, axis=0, keepdims=True)
    dca = jnp.sum(wqt * xt, axis=0, keepdims=True) + jnp.sum(wkvf * yt, axis=0, keepdims=True)
    dmod = jnp.concatenate([dsa, dca], axis=1)
    for n in range(2 * D // 128):
        dwmod_v[:, n * 128:(n + 1) * 128] = (sccol_ref[...] * dmod[:, n * 128:(n + 1) * 128]).astype(bf16)
    cp_dma.start()

    dsc = _dot_nt(_hilo_rows(dmod), wmod_ref[:, 0:2 * D])
    dsc = dsc + jnp.concatenate([dscb_ref[k] for k in range(4)], axis=1)
    dsc = dsc[0:1] + dsc[1:2]
    dc_ref[...] = (dsc * (sig_c * (1.0 + c * (1.0 - sig_c)))).astype(bf16)

    def fin_body(i, carry):
        rows = blk(i)
        dh1 = (_dot(wq_ref[...], dqt_ref[i]) + _dot(wkvc_ref[...], dkvc_ref[i])).T
        xhat, rstd = _ln(x_ref[rows, :].astype(f32))
        dx = dx1_ref[rows, :] + _ln_bwd(dh1 * (1.0 + modrow(1)), xhat, rstd)
        g_ref[rows, :] = dx.astype(bf16)
        dx_copy(i).start()
        return carry

    lax.fori_loop(0, NB, fin_body, 0)

    for i in range(NB):
        out_copy(i).wait()
        dx_copy(i).wait()
    cp_dw1.wait()
    cp_dw2.wait()
    cp_dwo.wait()
    cp_dmb.wait()
    cp_dma.wait()
    cp_dwq.wait()


@jax.jit
def pallas_adaLN_cond__grouped_kv_mqa__dense_activation_silu__prompt_kernel(
    A_x: jax.Array,
    A_wq: jax.Array,
    A_wk: jax.Array,
    A_wv: jax.Array,
    A_wo: jax.Array,
    B_x: jax.Array,
    B_w1: jax.Array,
    B_w2: jax.Array,
    c: jax.Array,
    w_mod: jax.Array,
    grad_out: jax.Array,
):
    del B_x
    x = A_x.reshape(S, D)
    g = grad_out.reshape(S, D)
    sds = jax.ShapeDtypeStruct
    out_shape = (
        sds((S, D), bf16), sds((S, D), bf16),
        sds((D, D), bf16), sds((DH, D), bf16), sds((DH, D), bf16), sds((D, D), bf16),
        sds((F, D), bf16), sds((F, D), bf16), sds((1, D), bf16), sds((D, 6 * D), bf16),
    )
    hbm = pl.BlockSpec(memory_space=pl.ANY)
    vm = pl.BlockSpec(memory_space=pltpu.VMEM)
    scratch = [
        pltpu.VMEM((S, D), bf16),
        pltpu.VMEM((S, D), bf16),
        pltpu.VMEM((D, D), bf16),
        pltpu.VMEM((D, D), bf16),
        pltpu.VMEM((F, D), bf16),
        pltpu.VMEM((F, D), bf16),
        pltpu.VMEM((D, 6 * D), bf16),
        pltpu.VMEM((S, D), bf16),
        pltpu.VMEM((D, D), bf16),
        pltpu.VMEM((D, D), bf16),
        pltpu.VMEM((F, D), bf16),
        pltpu.VMEM((F, D), bf16),
        pltpu.VMEM((D, 6 * D), bf16),
        pltpu.VMEM((8, 6 * D), f32),
        pltpu.VMEM((NB, D // 2, TQ), u32),
        pltpu.VMEM((8, S // 2, 32), u32),
        pltpu.VMEM((NB, 128, TQ), u32),
        pltpu.VMEM((H, S // 2, TQ), u32),
        pltpu.VMEM((2, S, TQ), f32),
        pltpu.VMEM((2, 8, TQ), f32),
        pltpu.VMEM((D, TQ), f32),
        pltpu.VMEM((H + 1, 16, TQ), u32),
        pltpu.VMEM((H, 8, TQ), f32),
        pltpu.VMEM((NB, D, TQ), bf16),
        pltpu.VMEM((S, D), f32),
        pltpu.VMEM((256, S), f32),
        pltpu.VMEM((F, D), f32),
        pltpu.VMEM((F, D), f32),
        pltpu.VMEM((D, D), f32),
        pltpu.VMEM((8, 6 * D), f32),
        pltpu.VMEM((D, D), bf16),
        pltpu.VMEM((NB, 64, TQ), bf16),
        pltpu.VMEM((2, S // 2, TQ), u32),
        pltpu.VMEM((D, 64), bf16),
        pltpu.VMEM((D, 128), f32),
        pltpu.VMEM((S, D), bf16),
        pltpu.VMEM((D, D), f32),
        pltpu.VMEM((D, TQ), f32),
        pltpu.VMEM((4, 16, D // 4), f32),
        pltpu.SemaphoreType.DMA((NSEM,)),
    ]
    outs = pl.pallas_call(
        _kernel,
        out_shape=out_shape,
        in_specs=[hbm, hbm, vm, vm, hbm, hbm, hbm, vm, hbm, hbm],
        out_specs=(hbm, hbm, hbm, vm, vm, hbm, hbm, hbm, vm, hbm),
        scratch_shapes=scratch,
        compiler_params=pltpu.CompilerParams(vmem_limit_bytes=124 * 1024 * 1024),
    )(x, A_wq, A_wk.T, A_wv.T, A_wo, B_w1.T, B_w2, c, w_mod, g)
    out, dx, dwq, dwkt, dwvt, dwo, dw1t, dw2, dc, dwmod = outs
    return (out.reshape(1, S, D), dx.reshape(1, S, D), dwq, dwkt.T, dwvt.T, dwo, dw1t.T, dw2, dc, dwmod)
```

```python
import math

import jax
import jax.numpy as jnp
from jax import lax
import jax.experimental.pallas as pl
import jax.experimental.pallas.tpu as pltpu

S, D, H, DH, F = 2048, 640, 32, 20, 1728
TQ = 256
NB = S // TQ
CK = 128
NCK = S // CK
HF = 8
HB = 8
FS = 512
QS = 160
EPS = 1e-5
f32, bf16, u32 = jnp.float32, jnp.bfloat16, jnp.uint32
LEAD = 4
SKEW = 3
NT = (((1,), (1,)), ((), ()))
SM_SCALE = DH ** (-0.5)
QSCALE = SM_SCALE * math.log2(math.e)
ONE_ROWS = ((30, 31), (30, 31), (30, 31), (0, 1))

SEM_X = 0
SEM_WMA, SEM_WMB, SEM_WQ, SEM_WO, SEM_W1, SEM_W2, SEM_G = range(NB, NB + 7)
SEM_OUT = NB + 7
SEM_DX = 2 * NB + 7
SEM_DWQ, SEM_DWO, SEM_DW1, SEM_DW2, SEM_DMA_, SEM_DMB = range(3 * NB + 7, 3 * NB + 13)
NSEM = 3 * NB + 13


def woff(rr):
    return 80 * (rr // 4) + 16 * (rr % 4)


def _pk(v):
    return pltpu.bitcast(v, u32)


def _upk(v):
    return pltpu.bitcast(v, bf16)


def _dot(a, b):
    return jnp.dot(a, b, preferred_element_type=f32)


def _dot_nt(a, b):
    return lax.dot_general(a, b, NT, preferred_element_type=f32)


def _ln(x):
    mu = jnp.mean(x, axis=-1, keepdims=True)
    xc = x - mu
    var = jnp.mean(xc * xc, axis=-1, keepdims=True)
    rstd = lax.rsqrt(var + EPS)
    return xc * rstd, rstd


def _ln_bwd(dxhat, xhat, rstd):
    m1 = jnp.mean(dxhat, axis=-1, keepdims=True)
    m2 = jnp.mean(dxhat * xhat, axis=-1, keepdims=True)
    return rstd * (dxhat - m1 - xhat * m2)


def _hilo_rows(v):
    hi = v.astype(bf16).astype(f32)
    r = lax.broadcasted_iota(jnp.int32, (16, v.shape[1]), 0)
    return jnp.where(r == 0, hi, jnp.where(r == 1, v - hi, 0.0)).astype(bf16)


def _colsum8(v):
    r, c = v.shape
    return jnp.sum(v.reshape(r // 8, 8, c), axis=0)


def _kernel(x_hbm, wq_hbm, wkt_ref, wvt_ref, wo_hbm, w1t_hbm, w2_hbm, c_ref, wmod_hbm, g_hbm,
            out_hbm, dx_hbm, dwq_hbm, dwkt_ref, dwvt_ref, dwo_hbm, dw1t_hbm, dw2_hbm, dc_ref, dwmod_hbm,
            x_ref, g_ref, wq_ref, wo_ref, w1t_ref, w2_ref, wmod_ref,
            out_v, dwq_v, dwo_v, dw1t_v, dw2_v, dwmod_v,
            mod_ref, qt_ref, kv_ref, kvt_ref, e_ref, s_ref, m_ref, ot_ref, gw_ref,
            linv_ref, dqt_ref, dx1_ref, dkv_ref, dw1t_acc, dw2_acc, dwo_acc, dmod_acc,
            wqt_ref, dkvc_ref, ds_ref, wkvc_ref, sccol_ref, xh_ref, xt_acc, qs_acc, dscb_ref, sems):

    def blk(i):
        return pl.ds(pl.multiple_of(i * TQ, TQ), TQ)

    def x_copy(i):
        return pltpu.make_async_copy(x_hbm.at[blk(i)], x_ref.at[blk(i)], sems.at[SEM_X + i])

    def out_copy(i):
        return pltpu.make_async_copy(out_v.at[blk(i)], out_hbm.at[blk(i)], sems.at[SEM_OUT + i])

    def dx_copy(i):
        return pltpu.make_async_copy(g_ref.at[blk(i)], dx_hbm.at[blk(i)], sems.at[SEM_DX + i])

    cp_wma = pltpu.make_async_copy(wmod_hbm.at[:, 0:2 * D], wmod_ref.at[:, 0:2 * D], sems.at[SEM_WMA])
    cp_wmb = pltpu.make_async_copy(wmod_hbm.at[:, 2 * D:6 * D], wmod_ref.at[:, 2 * D:6 * D], sems.at[SEM_WMB])
    cp_wq = pltpu.make_async_copy(wq_hbm, wq_ref, sems.at[SEM_WQ])
    cp_wo = pltpu.make_async_copy(wo_hbm, wo_ref, sems.at[SEM_WO])
    cp_w1 = pltpu.make_async_copy(w1t_hbm, w1t_ref, sems.at[SEM_W1])
    cp_w2 = pltpu.make_async_copy(w2_hbm, w2_ref, sems.at[SEM_W2])
    cp_g = pltpu.make_async_copy(g_hbm, g_ref, sems.at[SEM_G])
    cp_dwq = pltpu.make_async_copy(dwq_v, dwq_hbm, sems.at[SEM_DWQ])
    cp_dwo = pltpu.make_async_copy(dwo_v, dwo_hbm, sems.at[SEM_DWO])
    cp_dw1 = pltpu.make_async_copy(dw1t_v, dw1t_hbm, sems.at[SEM_DW1])
    cp_dw2 = pltpu.make_async_copy(dw2_v, dw2_hbm, sems.at[SEM_DW2])
    cp_dma = pltpu.make_async_copy(dwmod_v.at[:, 0:2 * D], dwmod_hbm.at[:, 0:2 * D], sems.at[SEM_DMA_])
    cp_dmb = pltpu.make_async_copy(dwmod_v.at[:, 2 * D:6 * D], dwmod_hbm.at[:, 2 * D:6 * D], sems.at[SEM_DMB])

    cp_wq.start()
    cp_wma.start()
    x_copy(0).start()

    def zero_body(k, carry):
        fr = pl.ds(pl.multiple_of(k * (F // 8), 8), F // 8)
        dr = pl.ds(pl.multiple_of(k * (D // 8), 8), D // 8)
        dkv_ref[pl.ds(pl.multiple_of(k * 32, 8), 32), :] = jnp.zeros((32, S), f32)
        dw1t_acc[fr, :] = jnp.zeros((F // 8, D), f32)
        dw2_acc[fr, :] = jnp.zeros((F // 8, D), f32)
        dwo_acc[dr, :] = jnp.zeros((D // 8, D), f32)
        xt_acc[dr, :] = jnp.zeros((D // 8, D), f32)
        qs_acc[dr, :] = jnp.zeros((D // 8, TQ), f32)
        return carry

    lax.fori_loop(0, 8, zero_body, 0)
    dmod_acc[...] = jnp.zeros_like(dmod_acc)
    gw_ref[H] = jnp.zeros((16, TQ), u32)

    c = c_ref[...].astype(f32)
    sig_c = jax.nn.sigmoid(c)
    sc = c * sig_c
    sc8 = jnp.broadcast_to(sc, (8, D)).astype(bf16)
    sccol_ref[...] = jnp.broadcast_to(sc, (128, D)).T

    r_i = lax.broadcasted_iota(jnp.int32, (64, DH), 0)
    d_i = lax.broadcasted_iota(jnp.int32, (64, DH), 1)
    selk = jnp.where(r_i == d_i, 1.0, 0.0).astype(bf16)
    selv = jnp.where(r_i == d_i + 32, 1.0, 0.0).astype(bf16)
    wkvct = (_dot(selk, wkt_ref[...]) + _dot(selv, wvt_ref[...])).astype(bf16)
    wkvc_ref[...] = wkvct.T
    sr = lax.broadcasted_iota(jnp.int32, (64, 256), 0)
    scn = lax.broadcasted_iota(jnp.int32, (64, 256), 1)
    shift = jnp.where(jnp.logical_and((scn // 128) == (sr // 32),
                                      (scn % 32) - 4 * ((scn % 128) // 32) == (sr % 32)), 1.0, 0.0)
    shift_t = shift.T.astype(bf16)
    shift = shift.astype(bf16)

    def ones_mask(idx):
        m = None
        for r in range(4):
            for o in ONE_ROWS[r]:
                t = idx == (128 + 32 * r + o)
                m = t if m is None else jnp.logical_or(m, t)
        return m

    colmask = ones_mask(lax.broadcasted_iota(jnp.int32, (TQ, 256), 1))
    rowmask = ones_mask(lax.broadcasted_iota(jnp.int32, (256, TQ), 0))

    cp_wq.wait()
    for i in range(1, NB):
        x_copy(i).start()

    def wqt_body(k, carry):
        cs = pl.ds(pl.multiple_of(k * 128, 128), 128)
        wqt_ref[cs, :] = wq_ref[:, cs].T
        return carry

    lax.fori_loop(0, D // 128, wqt_body, 0)
    cp_wma.wait()
    mod_ref[:, 0:2 * D] = _dot(sc8, wmod_ref[:, 0:2 * D])

    def modrow(k):
        return mod_ref[0:1, k * D:(k + 1) * D]

    def p0_ln(i):
        rows = blk(i)
        xhat, _ = _ln(x_ref[rows, :].astype(f32))
        xh_ref[rows, :] = xhat.astype(bf16)
        return (xhat * (1.0 + modrow(1)) + modrow(0)).astype(bf16)

    def p0_body(i, h1):
        @pl.when(i + 1 < NB)
        def _():
            x_copy(i + 1).wait()

        h1_next = p0_ln(jnp.minimum(i + 1, NB - 1))
        kvct = _dot_nt(wkvct, h1).astype(bf16)
        qt_ref.at[i][0:QS // 2, :] = _pk((_dot_nt(wqt_ref[0:QS, :], h1) * QSCALE).astype(bf16))
        kvt_ref.at[i][...] = _pk(jnp.where(rowmask, 1.0, _dot(shift_t, kvct)).astype(bf16))
        kv = _pk(jnp.where(colmask, 1.0, _dot(kvct.T, shift)).astype(bf16))
        rows2 = pl.ds(pl.multiple_of(i * (TQ // 2), TQ // 2), TQ // 2)
        for v in range(8):
            kv_ref[v, rows2, :] = kv[:, 32 * v:32 * v + 32]
        qt_ref.at[i][QS // 2:D // 2, :] = _pk((_dot_nt(wqt_ref[QS:D, :], h1) * QSCALE).astype(bf16))
        return h1_next

    x_copy(0).wait()
    h1_first = p0_ln(0)
    cp_wmb.start()
    cp_wo.start()
    cp_w1.start()
    cp_w2.start()
    cp_g.start()
    lax.fori_loop(0, NB, p0_body, h1_first)

    wrow = lax.broadcasted_iota(jnp.int32, (32, TQ), 0)

    def head_mask(r):
        return jnp.logical_and(wrow >= 4 * r, wrow < 4 * r + DH)

    def kvt_chunk(v, j):
        return _upk(kvt_ref[j // 2, 16 * v:16 * v + 16, (j % 2) * CK:(j % 2 + 1) * CK])

    def scores_chunk(j, r, qwin, slot, mrun):
        ks = slice(j * CK, (j + 1) * CK)
        s = _dot(_upk(kv_ref[r, j * CK // 2:(j + 1) * CK // 2, :]), qwin)
        s_ref[slot, ks, :] = s
        cm = jnp.max(s.reshape(CK // 8, 8, TQ), axis=0)
        return cm if mrun is None else jnp.maximum(mrun, cm)

    def finish_max(mrun):
        return jnp.broadcast_to(jnp.max(mrun, axis=0, keepdims=True), (8, TQ))

    m_ref[...] = jnp.full((2, 8, TQ), -jnp.inf, f32)

    def pro_body(q, carry):
        hd = q // (NCK // LEAD)
        k0 = (q % (NCK // LEAD)) * (LEAD * CK)
        qwin = _upk(qt_ref[0, pl.ds(pl.multiple_of(hd * 8, 8), 16), :])
        kk = _upk(kv_ref[hd, pl.ds(pl.multiple_of(k0 // 2, 8), LEAD * CK // 2), :])
        sc_ = _dot(kk, qwin)
        s_ref[hd, pl.ds(pl.multiple_of(k0, 8), LEAD * CK), :] = sc_
        m_ref[hd] = jnp.maximum(m_ref[hd], jnp.max(sc_.reshape(LEAD * CK // 8, 8, TQ), axis=0))
        return carry

    lax.fori_loop(0, NCK // LEAD + 1, pro_body, 0)
    m_ref[0] = finish_max(m_ref[0])

    def assemble(wins):
        pieces = []
        for p in range(5):
            t = None
            if p <= 3:
                t = wins[p][0:16]
            if p >= 1:
                u = wins[p - 1][16:32]
                t = u if t is None else t + u
            pieces.append(t)
        return jnp.concatenate(pieces, axis=0)

    def ds_produce(h, hg, r, j):
        ks = slice(j * CK, (j + 1) * CK)
        ks2 = slice(j * CK // 2, (j + 1) * CK // 2)
        gw = _upk(gw_ref[hg])
        e = _upk(e_ref[h, ks2, :])
        dkv_ref[128 + 32 * r:128 + 32 * r + 32, ks] += _dot_nt(gw, e)
        gt = _dot(_upk(kv_ref[4 + r, ks2, :]), gw)
        ds_ref[r % 2, ks2, :] = _pk((e.astype(f32) * gt).astype(bf16))

    def block_body(i, carry):
        rows = blk(i)

        def fwd_group(g, carry):
            base = pl.multiple_of(g * (20 * HF), 16)
            base2 = pl.multiple_of(g * (10 * HF), 8)
            last = g == H // HF - 1
            nb_i = jnp.where(last, jnp.minimum(i + 1, NB - 1), i)
            nbase2 = pl.multiple_of(jnp.where(last, 0, base2 + 10 * HF), 8)

            def q_window(rr):
                if rr < HF:
                    return _upk(qt_ref[i, pl.ds(base2 + woff(rr) // 2, 16), :])
                return _upk(qt_ref[nb_i, pl.ds(nbase2 + woff(rr - HF) // 2, 16), :])

            m_head = {0: m_ref[0]}
            mrun = m_ref[1]
            wins = []
            oacc = None
            for t in range(HF * NCK):
                rr, j = divmod(t, NCK)
                r = rr % 4
                ra, ja = divmod(t + NCK + LEAD, NCK)
                mrun = scores_chunk(ja, ra % 4, q_window(ra), ra % 2, mrun)
                if ja == NCK - 1:
                    m_head[ra] = finish_max(mrun)
                    mrun = None
                h = g * HF + rr
                ks = slice(j * CK, (j + 1) * CK)
                ks2 = slice(j * CK // 2, (j + 1) * CK // 2)
                e = jnp.exp2(s_ref[r % 2, ks, :] - m_head[rr][0:1, :]).astype(bf16)
                e_ref[h, ks2, :] = _pk(e)
                po = _dot(kvt_chunk(4 + r, j), e)
                oacc = po if oacc is None else oacc + po
                if j == NCK - 1:
                    lr = ONE_ROWS[r][0]
                    linv = 1.0 / oacc[lr:lr + 1, :]
                    linv_ref[h] = jnp.broadcast_to(linv, (8, TQ))
                    wins.append(jnp.where(head_mask(r), oacc * linv, 0.0))
                    oacc = None
                    if r == 3:
                        ot_ref[pl.ds(base + 80 * (rr // 4), 80), :] = assemble(wins)
                        wins = []
            m_ref[0] = m_head[HF]
            m_ref[1] = mrun
            return carry

        lax.fori_loop(0, H // HF, fwd_group, 0)

        @pl.when(i == 0)
        def _():
            cp_wmb.wait()
            cp_wo.wait()
            cp_w1.wait()
            cp_w2.wait()
            cp_g.wait()

            def modb(k, carry):
                cs = pl.ds(pl.multiple_of(k * D, 128), D)
                mod_ref[:, cs] = _dot(sc8, wmod_ref[:, cs])
                return carry

            lax.fori_loop(2, 6, modb, 0)

        ga, sb, cb, gb = modrow(2), modrow(3), modrow(4), modrow(5)
        g = g_ref[rows, :].astype(f32)
        df = (g * gb).astype(bf16)
        dsl_a = _dot_nt(df, w2_ref[0:FS, :])
        ot = ot_ref[...]
        otb = ot.astype(bf16)
        a = _dot(otb.T, wo_ref[...])
        dsl = jnp.concatenate([dsl_a, _dot_nt(df, w2_ref[FS:F, :])], axis=1)
        x1 = x_ref[rows, :].astype(f32) + ga * a
        xhat2, rstd2 = _ln(x1)
        h2 = (xhat2 * (1.0 + cb) + sb).astype(bf16)
        u = _dot_nt(h2, w1t_ref[...])
        sig = 0.5 * jnp.tanh(0.5 * u) + 0.5
        sl = (u * sig).astype(bf16)
        du = (dsl * (sig * (1.0 + u * (1.0 - sig)))).astype(bf16)
        dh2 = _dot(du, w1t_ref[...])
        f = _dot(sl, w2_ref[...])
        out_v[rows, :] = (x1 + gb * f).astype(bf16)
        out_copy(i).start()
        dmod_acc[:, 5 * D:6 * D] += _colsum8(g * f)
        dmod_acc[:, 3 * D:4 * D] += _colsum8(dh2)
        dmod_acc[:, 4 * D:5 * D] += _colsum8(dh2 * xhat2)
        dx1 = g + _ln_bwd(dh2 * (1.0 + cb), xhat2, rstd2)
        dx1_ref[rows, :] = dx1
        dmod_acc[:, 2 * D:3 * D] += _colsum8(dx1 * a)
        da = (dx1 * ga).astype(bf16)
        dot = _dot_nt(wo_ref[...], da)
        dw2_acc[...] += _dot(sl.T, df)
        dw1t_acc[...] += _dot(du.T, h2)
        for h in range(H):
            gg, r = divmod(h, 4)
            wsl = slice(80 * gg + 16 * r, 80 * gg + 16 * r + 32)
            dow = jnp.where(head_mask(r), dot[wsl, :], 0.0)
            linv = linv_ref[h][0:1, :]
            delta = jnp.sum(dow * ot[wsl, :], axis=0, keepdims=True) * linv
            d_hi = delta.astype(bf16).astype(f32)
            d_lo = delta - d_hi
            r0, r1 = ONE_ROWS[r]
            gw = dow * linv
            gw = jnp.where(wrow == r0, -d_hi, gw)
            gw = jnp.where(wrow == r1, -d_lo, gw)
            gw_ref.at[h][...] = _pk(gw.astype(bf16))
        for j in range(SKEW):
            ds_produce(0, 0, 0, j)
        dwo_acc[...] += _dot(otb, da)

        @pl.when(i == NB - 1)
        def _():
            dmb = jnp.sum(dmod_acc[:, 2 * D:6 * D], axis=0, keepdims=True)
            dmod_acc[0:1, 2 * D:6 * D] = dmb
            dmb2 = _hilo_rows(dmb)

            def stage(k, carry):
                fr = pl.ds(pl.multiple_of(k * (F // 4), 16), F // 4)
                dr = pl.ds(pl.multiple_of(k * (D // 4), 16), D // 4)
                dw1t_v[fr, :] = dw1t_acc[fr, :].astype(bf16)
                dw2_v[fr, :] = dw2_acc[fr, :].astype(bf16)
                dwo_v[dr, :] = dwo_acc[dr, :].astype(bf16)
                dscb_ref[k] = _dot_nt(dmb2, wmod_ref[dr, 2 * D:6 * D])
                scc = sccol_ref[dr, :]
                for n in range(2 * D // 128, 6 * D // 128):
                    cs = slice(n * 128, (n + 1) * 128)
                    dwmod_v[dr, cs] = (scc * dmod_acc[0:1, cs]).astype(bf16)
                return carry

            lax.fori_loop(0, 4, stage, 0)
            cp_dw1.start()
            cp_dw2.start()
            cp_dwo.start()
            cp_dmb.start()

        def bwd_group(g, carry):
            base = pl.multiple_of(g * (20 * HB), 16)
            base2 = pl.multiple_of(g * (10 * HB), 8)
            hnext = jnp.minimum(g * HB + HB, H - 4)
            wins = []
            dq = None
            for t in range(HB * NCK):
                rp, jp = divmod(t + SKEW, NCK)
                ds_produce(g * HB + rp if rp < HB else hnext, g * HB + rp, rp % 4, jp)
                rr, j = divmod(t, NCK)
                r = rr % 4
                ks = slice(j * CK, (j + 1) * CK)
                ks2 = slice(j * CK // 2, (j + 1) * CK // 2)
                qwin = _upk(qt_ref[i, pl.ds(base2 + woff(rr) // 2, 16), :])
                ds = _upk(ds_ref[r % 2, ks2, :])
                dkv_ref[32 * r:32 * r + 32, ks] += _dot_nt(qwin, ds)
                pq = _dot(kvt_chunk(r, j), ds)
                dq = pq if dq is None else dq + pq
                if j == NCK - 1:
                    wins.append(jnp.where(head_mask(r), dq * SM_SCALE, 0.0))
                    dq = None
                    if r == 3:
                        dqt_ref[i, pl.ds(base + 80 * (rr // 4), 80), :] = assemble(wins).astype(bf16)
                        wins = []
            return carry

        lax.fori_loop(0, H // HB, bwd_group, 0)
        return carry

    lax.fori_loop(0, NB, block_body, 0)

    dkt = None
    dvt = None
    for r in range(4):
        a_ = dkv_ref[36 * r:36 * r + DH, :]
        b_ = dkv_ref[128 + 36 * r:128 + 36 * r + DH, :]
        dkt = a_ if dkt is None else dkt + a_
        dvt = b_ if dvt is None else dvt + b_
    dkv_ref[0:64, :] = jnp.zeros((64, S), f32)
    dkv_ref[0:DH, :] = dkt * (SM_SCALE / QSCALE)
    dkv_ref[32:32 + DH, :] = dvt
    dkvc = dkv_ref[0:64, :].astype(bf16)
    for i in range(NB):
        dkvc_ref[i] = dkvc[:, i * TQ:(i + 1) * TQ]

    sa, ca = modrow(0), modrow(1)
    ckv = jnp.sum(dkvc.astype(f32), axis=1, keepdims=True)

    def x_body(i, yt):
        dqt = dqt_ref[i]
        xh = xh_ref[blk(i), :]
        xt_acc[...] += _dot(dqt, xh)
        qs_acc[...] += dqt.astype(f32)
        return yt + _dot(dkvc_ref[i], xh)

    yt = lax.fori_loop(0, NB, x_body, jnp.zeros((64, D), f32))
    dwkvt = yt * (1.0 + ca) + ckv * sa
    dwkt_ref[...] = dwkvt[0:DH, :].astype(bf16)
    dwvt_ref[...] = dwkvt[32:32 + DH, :].astype(bf16)
    wkvf = wkvct.astype(f32)

    def dwq_body(k, carry):
        sa8, ca8 = carry
        js = pl.ds(pl.multiple_of(k * 128, 128), 128)
        xt = xt_acc[js, :]
        cq = jnp.sum(qs_acc[js, :], axis=1, keepdims=True)
        dwq_v[:, js] = (xt * (1.0 + ca) + cq * sa).T.astype(bf16)
        wqt = wqt_ref[js, :].astype(f32)
        return sa8 + _colsum8(wqt * cq), ca8 + _colsum8(wqt * xt)

    sa8, ca8 = lax.fori_loop(0, D // 128, dwq_body, (_colsum8(wkvf * ckv), _colsum8(wkvf * yt)))
    cp_dwq.start()
    dmod = jnp.concatenate([jnp.sum(sa8, axis=0, keepdims=True),
                            jnp.sum(ca8, axis=0, keepdims=True)], axis=1)

    dm2 = _hilo_rows(dmod)

    def dwm_body(k, carry):
        dr = pl.ds(pl.multiple_of(k * (D // 4), 16), D // 4)
        dscb_ref[k] += _dot_nt(dm2, wmod_ref[dr, 0:2 * D])
        scc = sccol_ref[dr, :]
        for n in range(2 * D // 128):
            cs = slice(n * 128, (n + 1) * 128)
            dwmod_v[dr, cs] = (scc * dmod[:, cs]).astype(bf16)
        return carry

    lax.fori_loop(0, 4, dwm_body, 0)
    cp_dma.start()

    dsc = jnp.concatenate([dscb_ref[k] for k in range(4)], axis=1)
    dsc = dsc[0:1] + dsc[1:2]
    dc_ref[...] = (dsc * (sig_c * (1.0 + c * (1.0 - sig_c)))).astype(bf16)

    def fin_body(i, carry):
        rows = blk(i)
        dh1 = (_dot(wq_ref[...], dqt_ref[i]) + _dot(wkvc_ref[...], dkvc_ref[i])).T
        xhat, rstd = _ln(x_ref[rows, :].astype(f32))
        dx = dx1_ref[rows, :] + _ln_bwd(dh1 * (1.0 + modrow(1)), xhat, rstd)
        g_ref[rows, :] = dx.astype(bf16)
        dx_copy(i).start()
        return carry

    lax.fori_loop(0, NB, fin_body, 0)

    for i in range(NB):
        out_copy(i).wait()
        dx_copy(i).wait()
    cp_dw1.wait()
    cp_dw2.wait()
    cp_dwo.wait()
    cp_dmb.wait()
    cp_dma.wait()
    cp_dwq.wait()


@jax.jit
def pallas_adaLN_cond__grouped_kv_mqa__dense_activation_silu__prompt_kernel(
    A_x: jax.Array,
    A_wq: jax.Array,
    A_wk: jax.Array,
    A_wv: jax.Array,
    A_wo: jax.Array,
    B_x: jax.Array,
    B_w1: jax.Array,
    B_w2: jax.Array,
    c: jax.Array,
    w_mod: jax.Array,
    grad_out: jax.Array,
):
    del B_x
    x = A_x.reshape(S, D)
    g = grad_out.reshape(S, D)
    sds = jax.ShapeDtypeStruct
    out_shape = (
        sds((S, D), bf16), sds((S, D), bf16),
        sds((D, D), bf16), sds((DH, D), bf16), sds((DH, D), bf16), sds((D, D), bf16),
        sds((F, D), bf16), sds((F, D), bf16), sds((1, D), bf16), sds((D, 6 * D), bf16),
    )
    hbm = pl.BlockSpec(memory_space=pl.ANY)
    vm = pl.BlockSpec(memory_space=pltpu.VMEM)
    scratch = [
        pltpu.VMEM((S, D), bf16),
        pltpu.VMEM((S, D), bf16),
        pltpu.VMEM((D, D), bf16),
        pltpu.VMEM((D, D), bf16),
        pltpu.VMEM((F, D), bf16),
        pltpu.VMEM((F, D), bf16),
        pltpu.VMEM((D, 6 * D), bf16),
        pltpu.VMEM((S, D), bf16),
        pltpu.VMEM((D, D), bf16),
        pltpu.VMEM((D, D), bf16),
        pltpu.VMEM((F, D), bf16),
        pltpu.VMEM((F, D), bf16),
        pltpu.VMEM((D, 6 * D), bf16),
        pltpu.VMEM((8, 6 * D), f32),
        pltpu.VMEM((NB, D // 2, TQ), u32),
        pltpu.VMEM((8, S // 2, 32), u32),
        pltpu.VMEM((NB, 128, TQ), u32),
        pltpu.VMEM((H, S // 2, TQ), u32),
        pltpu.VMEM((2, S, TQ), f32),
        pltpu.VMEM((2, 8, TQ), f32),
        pltpu.VMEM((D, TQ), f32),
        pltpu.VMEM((H + 1, 16, TQ), u32),
        pltpu.VMEM((H, 8, TQ), f32),
        pltpu.VMEM((NB, D, TQ), bf16),
        pltpu.VMEM((S, D), f32),
        pltpu.VMEM((256, S), f32),
        pltpu.VMEM((F, D), f32),
        pltpu.VMEM((F, D), f32),
        pltpu.VMEM((D, D), f32),
        pltpu.VMEM((8, 6 * D), f32),
        pltpu.VMEM((D, D), bf16),
        pltpu.VMEM((NB, 64, TQ), bf16),
        pltpu.VMEM((2, S // 2, TQ), u32),
        pltpu.VMEM((D, 64), bf16),
        pltpu.VMEM((D, 128), f32),
        pltpu.VMEM((S, D), bf16),
        pltpu.VMEM((D, D), f32),
        pltpu.VMEM((D, TQ), f32),
        pltpu.VMEM((4, 16, D // 4), f32),
        pltpu.SemaphoreType.DMA((NSEM,)),
    ]
    outs = pl.pallas_call(
        _kernel,
        out_shape=out_shape,
        in_specs=[hbm, hbm, vm, vm, hbm, hbm, hbm, vm, hbm, hbm],
        out_specs=(hbm, hbm, hbm, vm, vm, hbm, hbm, hbm, vm, hbm),
        scratch_shapes=scratch,
        compiler_params=pltpu.CompilerParams(vmem_limit_bytes=124 * 1024 * 1024),
    )(x, A_wq, A_wk.T, A_wv.T, A_wo, B_w1.T, B_w2, c, w_mod, g)
    out, dx, dwq, dwkt, dwvt, dwo, dw1t, dw2, dc, dwmod = outs
    return (out.reshape(1, S, D), dx.reshape(1, S, D), dwq, dwkt.T, dwvt.T, dwo, dw1t.T, dw2, dc, dwmod)
```
